```python
import os as _os
_os.environ.setdefault('JAX_PLATFORMS', 'cpu')
import jax
import jax.numpy as jnp

def _softmax(x, axis=-1):
    return jax.nn.softmax(x, axis=axis)

def _gelu(x):
    return jax.nn.gelu(x, approximate=True)

def _silu(x):
    return jax.nn.silu(x)

def _sigmoid(x):
    return jax.nn.sigmoid(x)

def _layernorm(x, axis=-1, eps=1e-05):
    m = jnp.mean(x, axis=axis, keepdims=True)
    v = jnp.var(x, axis=axis, keepdims=True)
    return (x - m) / jnp.sqrt(v + eps)

def _scatter_add(tgt, idx, src, axis=0):
    return tgt.at[idx].add(src)

def _segment_sum(src, seg, n):
    return jax.ops.segment_sum(src, seg, n)

class _Rng:

    def __init__(self, key):
        self._k = key

    def _next(self):
        self._k, sub = jax.random.split(self._k)
        return sub

    def normal(self, shape):
        return jax.random.normal(self._next(), shape, dtype=jnp.bfloat16)

    def randint(self, lo, hi, shape):
        return jax.random.randint(self._next(), shape, lo, hi, dtype=jnp.int32)

    def uniform(self, shape, lo=0.0, hi=1.0):
        return jax.random.uniform(self._next(), shape, jnp.bfloat16, lo, hi)

    def permutation(self, n):
        return jax.random.permutation(self._next(), n)
kernel_name = 'sequential_preLN__memory_aug_recurrent_mem_tr__mixer_token_mlp__prompt'

def setup_inputs():
    _rng = _Rng(jax.random.key(int.from_bytes(__import__("os").urandom(4), "little")))
    _w = lambda a: (lambda t: t.astype(jnp.bfloat16) if jnp.issubdtype(t.dtype, jnp.floating) else t)(jnp.asarray(a))

    def _A_setup():
        B, S, Dm = (1, 2048, 448)
        H, Dh = (16, 256)
        M, seg = (8, 32)
        seg = min(seg, S)
        S = S // seg * seg
        return {'x': _w((lambda *s: _rng.normal(s) * 0.05)(B, S, Dm)), 'mem0': _w((lambda *s: _rng.normal(s) * 0.2)(B, M, Dm)), 'Wq': _w((lambda *s: _rng.normal(s) * 1.6)(Dm, H, Dh) * Dm ** (-0.5)), 'Wk': _w((lambda *s: _rng.normal(s) * 1.6)(Dm, H, Dh) * Dm ** (-0.5)), 'Wv': _w((lambda *s: _rng.normal(s) * 0.2)(Dm, H, Dh) * Dm ** (-0.5)), 'Wo': _w((lambda *s: _rng.normal(s) * 0.2)(H, Dh, Dm) * (H * Dh) ** (-0.5)), 'seg_len': seg}
    _A_in = _A_setup()

    def _B_setup():
        B, S, D, F = (1, 2048, 448, 1792)
        return {'x': _w((lambda *s: _rng.normal(s) * 0.05)(B, S, D)), 'w1': _w((lambda *s: _rng.normal(s) * 0.2)(S, F) * S ** (-0.5)), 'b1': _w((lambda *s: _rng.normal(s) * 0.2)(F) * 0.02), 'w2': _w((lambda *s: _rng.normal(s) * 0.2)(F, S) * F ** (-0.5)), 'b2': _w((lambda *s: _rng.normal(s) * 0.05)(S) * 0.02)}
    _B_in = _B_setup()
    return {'A_x': _A_in['x'], 'A_mem0': _A_in['mem0'], 'A_Wq': _A_in['Wq'], 'A_Wk': _A_in['Wk'], 'A_Wv': _A_in['Wv'], 'A_Wo': _A_in['Wo'], 'A_seg_len': _A_in['seg_len'], 'B_x': _B_in['x'], 'B_w1': _B_in['w1'], 'B_b1': _B_in['b1'], 'B_w2': _B_in['w2'], 'B_b2': _B_in['b2']}

def reference(A_x, A_mem0, A_Wq, A_Wk, A_Wv, A_Wo, A_seg_len, B_x, B_w1, B_b1, B_w2, B_b2):

    def _A_ref(x, mem0, Wq, Wk, Wv, Wo, seg_len):
        B, S, Dm = x.shape
        H, Dh = (Wq.shape[1], Wq.shape[2])
        M = mem0.shape[1]
        scale = Dh ** (-0.5)
        n_seg = S // seg_len
        L = M + seg_len
        idx = jnp.arange(L)
        mask = (idx[:, None] < M) | (idx[:, None] >= idx[None, :])
        mem = mem0
        outs = []
        for s in range(n_seg):
            xs = x[:, s * seg_len:(s + 1) * seg_len, :].copy()
            h = jnp.concatenate([mem, xs], axis=1)
            q = jnp.einsum('btd,dhe->bhte', h, Wq)
            k = jnp.einsum('btd,dhe->bhte', h, Wk)
            v = jnp.einsum('btd,dhe->bhte', h, Wv)
            scores = jnp.einsum('bhqe,bhke->bhqk', q, k) * scale
            scores = jnp.where(mask[None, None], scores, -1000000000.0)
            p = _softmax(scores, axis=-1)
            o = jnp.einsum('bhqk,bhke->bhqe', p, v)
            o = jnp.einsum('bhte,hed->btd', o, Wo)
            mem = o[:, :M, :].copy()
            outs.append(o[:, M:, :])
        return jnp.concatenate(outs, axis=1)

    def _B_ref(x, w1, b1, w2, b2):
        B, S, D = x.shape
        h = _layernorm(x, axis=-1)
        u = jnp.einsum('bsd,sf->bdf', h, w1) + b1
        u = _gelu(u)
        y = jnp.einsum('bdf,fs->bds', u, w2) + b2
        return (lambda x, *d: x.transpose(*d))(y, 0, 2, 1)
    x = A_x
    h = x + _A_ref(_layernorm(x, axis=-1), A_mem0, A_Wq, A_Wk, A_Wv, A_Wo, A_seg_len)
    h2 = h + _B_ref(_layernorm(h, axis=-1), B_w1, B_b1, B_w2, B_b2)
    return h2
```

```python
import functools

import jax
import jax.numpy as jnp
from jax import lax
import jax.experimental.pallas as pl
import jax.experimental.pallas.tpu as pltpu

LANES = 128
SUB = 8
EPS = 1e-5
NEG = -1000000000.0
F32 = jnp.float32
BF16 = jnp.bfloat16
U32 = jnp.uint32
NT = (((1,), (1,)), ((), ()))

V_SPLIT = 4
SCOPES = False
U_LAG = 2
H_POS = 0
U_ROWS = True
X_POS = 3
TB = 512
R_T = True
HOSTCAST = False


class _NoScope:
    def __enter__(self):
        return None

    def __exit__(self, *a):
        return False


def _scope(name):
    return jax.named_scope(name) if SCOPES else _NoScope()


def _ln_cols(x):
    inv_n = 1.0 / x.shape[0]
    xc = x - jnp.sum(x, axis=0, keepdims=True) * inv_n
    var = jnp.sum(xc * xc, axis=0, keepdims=True) * inv_n
    return xc * lax.rsqrt(var + EPS)


def _gelu(u):
    c = 0.7978845608028654
    return 0.5 * u * (1.0 + jnp.tanh(c * (u + 0.044715 * (u * u * u))))


def _group_allreduce(x, op, lane):
    for sh in (1, 2, 4):
        up = pltpu.roll(x, sh, 1)
        down = pltpu.roll(x, LANES - sh, 1)
        x = op(x, jnp.where((lane & sh) != 0, up, down))
    return x


def _unpack_pair(words):
    even = lax.bitcast_convert_type(words << 16, F32)
    odd = lax.bitcast_convert_type(words & jnp.uint32(0xFFFF0000), F32)
    return even, odd


def _barrel(vs, lane, blk):
    n = len(vs)
    sh = 1
    while sh < n:
        hi = (lane & (blk * sh)) != 0
        nxt = []
        for r in range(n):
            a, b = vs[r], vs[(r + sh) % n]
            nxt.append(b if a is None else a if b is None else jnp.where(hi, b, a))
        vs = nxt
        sh *= 2
    return vs


def _pack(x):
    return pltpu.bitcast(x.astype(BF16), U32)


def _unpack(w):
    return pltpu.bitcast(w, BF16)


def _dot(a, b):
    return jnp.dot(a, b, preferred_element_type=F32)


def _dot_nt(a, b):
    return lax.dot_general(a, b, NT, preferred_element_type=F32)


def _kernel(xT_hbm, mem0_ref, wq_hbm, wk_hbm, wv_hbm, woT_hbm, w1_hbm, b1_ref, w2_hbm, b2_ref,
            outT_hbm,
            wq_s, wk_s, wv_s, wo_s, xT_s, w1_s, w2_s, WKm, WKs, WQ2, WVm, WVs, WB2,
            xn_s, attn_s, hT_s, hn_s, u_s, out_s, g_s, b2_s, wsem, xsem, w1sem, w2sem, osem, *, seg, scale):
    NB, D, _ = xT_s.shape
    S = NB * LANES
    HP = WKm.shape[0]
    M = mem0_ref.shape[0]
    L = M + seg
    F = u_s.shape[1]
    DF = D // LANES * LANES
    DR = D - DF
    NTILE = DF // LANES
    KG = L // SUB
    SPB = LANES // seg

    def pair_copy(i, src, dst, hp):
        w = src if HOSTCAST else src.bitcast(U32)
        return pltpu.make_async_copy(w.at[:, hp, :], dst.at[hp], wsem.at[i, hp])

    def qk_copies(hp):
        return [pair_copy(0, wk_hbm, wk_s, hp), pair_copy(1, wq_hbm, wq_s, hp)]

    def vo_copies(hp):
        two = pl.ds(2 * hp, 2)
        return [pair_copy(2, wv_hbm, wv_s, hp),
                pltpu.make_async_copy(woT_hbm.at[two], wo_s.at[two], wsem.at[3, hp])]

    def x_copy(b):
        c0 = b * LANES if isinstance(b, int) else pl.multiple_of(b * LANES, LANES)
        return pltpu.make_async_copy(xT_hbm.at[:, pl.ds(c0, LANES)], xT_s.at[b], xsem.at[b])

    def w1_copy(b):
        r0 = b * LANES if isinstance(b, int) else pl.multiple_of(b * LANES, LANES)
        return pltpu.make_async_copy(w1_hbm.at[pl.ds(r0, LANES)], w1_s.at[b], w1sem.at[b])

    w2_copy = pltpu.make_async_copy(w2_hbm, w2_s, w2sem.at[0])

    for hp in range(HP):
        for cp in qk_copies(hp):
            cp.start()

    def fuse_pair(l0, l1, r0, r1):
        z = jnp.zeros((DR, r0.shape[1]), r0.dtype)
        a0 = _dot_nt(l0, jnp.concatenate([r0, z], axis=0))
        a1 = _dot_nt(l1, jnp.concatenate([r1[:DF], z, r1[DF:]], axis=0))
        main = jnp.concatenate([a0[:DF, :DF], a1[:DF, :DF]], axis=1)
        rest = jnp.concatenate([a0[DF:, :DF], a1[DF:, :DF]], axis=0)
        return main, a0[:, DF:] + a1[:, DF:], rest

    def qk_body(hp, c):
        for cp in qk_copies(hp):
            cp.wait()
        for cp in vo_copies(hp):
            cp.start()
        q0, q1 = _unpack_pair(wq_s[hp])
        k0, k1 = _unpack_pair(wk_s[hp])
        main, shared, rest = fuse_pair(k0 * scale, k1 * scale, q0, q1)
        WKm[hp] = _pack(main)
        WKs[hp] = _pack(shared)
        WQ2[hp] = _pack(rest.T)
        return c

    def vo_body(hp, c):
        for cp in vo_copies(hp):
            cp.wait()
        v0, v1 = _unpack_pair(wv_s[hp])
        main, shared, rest = fuse_pair(v0, v1, wo_s[2 * hp], wo_s[2 * hp + 1])
        WVm[hp] = _pack(main)
        WVs[hp] = _pack(shared)
        WB2[hp] = _pack(rest)
        return c

    def x_norm(b):
        xn = _ln_cols(xT_s[b].astype(F32))
        xn_s[b] = jnp.concatenate([xn, xn[DF:]], axis=0).T

    with _scope('init'):
        x_copy(0).start()
        attn_s[0] = jnp.zeros(attn_s.shape[1:], F32)
        hn_s[...] = jnp.zeros(hn_s.shape, hn_s.dtype)
        u_s[...] = jnp.broadcast_to(b1_ref[...].astype(F32).reshape(1, F), u_s.shape)
        b2_s[...] = b2_ref[...].astype(F32).reshape(1, S)
    with _scope('qk'):
        lax.fori_loop(0, HP, qk_body, 0)
    with _scope('xn'):
        x_copy(1).start()
        w1_copy(0).start()
        x_copy(0).wait()
        x_norm(0)
    with _scope('vo'):
        lax.fori_loop(0, HP, vo_body, 0)

    def cat_pairs(ref):
        return _unpack(jnp.concatenate([ref[p] for p in range(HP)], axis=1))

    def segment(xs, mem):
        row = lax.broadcasted_iota(jnp.int32, (L, LANES), 0)
        lane = lax.broadcasted_iota(jnp.int32, (L, LANES), 1)
        lo = lane < DR

        def stack(heads):
            return jnp.concatenate(
                [h[g * SUB:(g + 1) * SUB] for g in range(KG) for h in heads], axis=0)

        def split_main(parts):
            return [p[:, j * DF:(j + 1) * DF] for p in parts for j in range(2)]

        def split_shared(sh):
            out = []
            for p in range(HP):
                t = sh[:, p * LANES:(p + 1) * LANES]
                out += [jnp.where(lo, t, 0.0), jnp.where(lo, 0.0, t)]
            return out

        hs = jnp.concatenate([mem, xs], axis=0)
        hm, hd, ht = hs[:, :DF], hs[:, :D], hs[:, DF:]
        q2 = _dot(hm, cat_pairs(WQ2))
        tl, th = jnp.where(lo, ht, 0.0), jnp.where(lo, 0.0, ht)
        zero = jnp.zeros((2 * SUB, LANES), F32)
        yblk = [jnp.concatenate([tl[g * SUB:(g + 1) * SUB], th[g * SUB:(g + 1) * SUB]], axis=0)
                for g in range(KG)] + [zero] * (HP - KG)
        km = [_dot(hm, _unpack(WKm[p])) for p in range(HP // 2)]
        q2s = jnp.concatenate([q2[:, p * LANES:(p + 1) * LANES] for p in range(HP)], axis=0)
        ycat = jnp.concatenate(yblk, axis=0)
        r = _dot(q2s, ycat.T.astype(BF16)) if R_T else _dot_nt(q2s, ycat.astype(BF16))
        rr = [r[p * L:(p + 1) * L] for p in range(HP)]
        rr = [pltpu.roll(t, 2 * SUB * p, 1) if p else t for p, t in enumerate(rr)]
        ww = _barrel(rr, lane, 2 * SUB)
        s2 = [ww[(-g) % HP] for g in range(KG)]
        s2 = [pltpu.roll(t, LANES - 2 * SUB * g, 1) if g else t for g, t in enumerate(s2)]
        km += [_dot(hm, _unpack(WKm[p])) for p in range(HP // 2, HP)]
        ks = _dot(hd, cat_pairs(WKs))
        kst = jnp.concatenate([stack(split_main(km)), stack(split_shared(ks))], axis=1)
        vm = [_dot(hm, _unpack(WVm[p])) for p in range(V_SPLIT)]
        sc = _dot(hs, kst.T.astype(BF16))
        vm += [_dot(hm, _unpack(WVm[p])) for p in range(V_SPLIT, HP)]
        tiles = []
        for g in range(KG):
            key = g * SUB + (lane & (SUB - 1))
            t = sc[:, g * LANES:(g + 1) * LANES] + s2[g]
            tiles.append(jnp.where((row < M) | (row >= key), t, NEG))
        mx = _group_allreduce(functools.reduce(jnp.maximum, tiles), jnp.maximum, lane)
        ex = [jnp.exp(t - mx) for t in tiles]
        inv = 1.0 / _group_allreduce(functools.reduce(jnp.add, ex), jnp.add, lane)
        prob = [e * inv for e in ex]
        vs = _dot(hd, cat_pairs(WVs))
        pp = [pltpu.roll(t, 2 * SUB * g, 1) if g else t for g, t in enumerate(prob)]
        uu = _barrel(pp + [None] * (HP - KG), lane, 2 * SUB)
        px = []
        for p in range(HP):
            y = jnp.concatenate([yblk[(j - p) % HP] for j in range(HP)], axis=0)
            px.append(_dot(uu[(-p) % HP], y.astype(BF16)))
        pc = jnp.concatenate(prob, axis=1)
        om = _dot(pc, stack(split_main(vm)).astype(BF16))
        wb2 = _unpack(jnp.concatenate([WB2[p] for p in range(HP)], axis=0))
        om = om + _dot(jnp.concatenate(px, axis=1), wb2)
        tail = _dot(pc, stack(split_shared(vs)).astype(BF16))
        o = jnp.concatenate([om, tail + pltpu.roll(tail, DR, 1)], axis=1)
        return o[:M], o[M:]

    def mixer_input(b, slot):
        hT = xT_s[b].astype(F32) + attn_s[slot].T[:D]
        hT_s[b] = hT
        return _ln_cols(_ln_cols(hT))

    def mix_in(hn, b, j):
        w = w1_s[b]
        if U_ROWS:
            rows = slice(j * D // SPB, (j + 1) * D // SPB)
            u_s[rows, :] += _dot(hn[rows], w)
        else:
            bounds = [0, 512, 1024, 1408, 1792]
            cols = slice(bounds[j], bounds[j + 1])
            u_s[:, cols] += _dot(hn, w[:, cols])

    def block_body(b, mem):
        w1_copy(b).wait()

        @pl.when(b + 1 < NB)
        def _():
            x_copy(b + 1).wait()
            w1_copy(b + 1).start()

        @pl.when(b + 2 < NB)
        def _():
            x_copy(b + 2).start()

        @pl.when(b == 0)
        def _():
            w2_copy.start()

        prev = jnp.maximum(b - 1, 0)
        if U_LAG == 2:
            hn = hn_s[...]
            ublk = jnp.maximum(b - 2, 0)
        for j in range(SPB):
            xs = xn_s[b, j * seg:(j + 1) * seg, :]
            if j == H_POS:
                hn_new = jnp.where(b > 0, mixer_input(prev, b), 0.0).astype(BF16)
                if U_LAG == 1:
                    hn, ublk = hn_new, prev
            if j == X_POS:
                nxt = jnp.minimum(b + 1, NB - 1)
                xn = _ln_cols(xT_s[nxt].astype(F32))
                xn_s[nxt] = jnp.concatenate([xn, xn[DF:]], axis=0).T
            mem, att = segment(xs, mem)
            attn_s[b + 1, j * seg:(j + 1) * seg, :] = att
            mix_in(hn, ublk, j)
        if U_LAG == 2:
            hn_s[...] = hn_new
        return mem

    m0 = mem0_ref[...].astype(F32)
    with _scope('main'):
        lax.fori_loop(0, NB, block_body, jnp.concatenate([m0, m0[:, DF:]], axis=1))

    with _scope('mlp'):
        hn = mixer_input(NB - 1, NB).astype(BF16)
        FB = 256
        if U_LAG == 2:
            hn = jnp.concatenate([hn_s[...], hn], axis=1)
            w = jnp.concatenate([w1_s[NB - 2], w1_s[NB - 1]], axis=0)
        else:
            w = w1_s[NB - 1]
        g = jnp.concatenate(
            [_gelu(u_s[:, f:f + FB] + _dot(hn, w[:, f:f + FB])).astype(BF16) for f in range(0, F, FB)],
            axis=1)
        w2_copy.wait()
        g_s[...] = g

        def out_copy(t):
            c0 = t * TB if isinstance(t, int) else pl.multiple_of(t * TB, TB)
            return pltpu.make_async_copy(out_s.at[:, pl.ds(c0, TB)], outT_hbm.at[:, pl.ds(c0, TB)], osem.at[t])


        def out_body(t, c):
            cols = pl.ds(pl.multiple_of(t * TB, TB), TB)
            y = _dot(g_s[...], w2_s[:, cols])
            nb = TB // LANES
            h = jnp.concatenate([hT_s[t * nb + j] for j in range(nb)], axis=1)
            out_s[:, cols] = (h + (y + b2_s[:, cols])).astype(out_s.dtype)
            out_copy(t).start()
            return c
        lax.fori_loop(0, S // TB, out_body, 0)
    with _scope('out_wait'):
        for t in range(S // TB):
            out_copy(t).wait()


def pallas_sequential_preLN__memory_aug_recurrent_mem_tr__mixer_token_mlp__prompt_kernel(A_x, A_mem0, A_Wq, A_Wk, A_Wv, A_Wo, A_seg_len, B_x, B_w1, B_b1, B_w2, B_b2):
    del B_x
    B, S, D = A_x.shape
    _, H, E = A_Wq.shape
    M = A_mem0.shape[1]
    F = B_w1.shape[1]
    seg = 32
    HP = H // 2
    DP = -(-D // LANES) * LANES
    DF = DP - LANES
    NB = S // LANES
    hbm = pl.BlockSpec(memory_space=pl.ANY)

    def hc(a):
        if not HOSTCAST:
            return a
        u = lax.bitcast_convert_type(a, jnp.uint16).astype(U32)
        return u[:, 0::2] | (u[:, 1::2] << 16)
    vmem = pl.BlockSpec(memory_space=pltpu.VMEM)
    outT = pl.pallas_call(
        functools.partial(_kernel, seg=seg, scale=E ** -0.5),
        out_shape=jax.ShapeDtypeStruct((D, S), A_x.dtype),
        in_specs=[hbm, vmem, hbm, hbm, hbm, hbm, hbm, vmem, hbm, vmem],
        out_specs=hbm,
        scratch_shapes=[
            pltpu.VMEM((HP, D, E), U32),
            pltpu.VMEM((HP, D, E), U32),
            pltpu.VMEM((HP, D, E), U32),
            pltpu.VMEM((H, D, E), BF16),
            pltpu.VMEM((NB, D, LANES), BF16),
            pltpu.VMEM((NB, LANES, F), BF16),
            pltpu.VMEM((F, S), BF16),
            pltpu.VMEM((HP, DF // 2, 2 * DF), U32),
            pltpu.VMEM((HP, D // 2, LANES), U32),
            pltpu.VMEM((HP, DF // 2, LANES), U32),
            pltpu.VMEM((HP, DF // 2, 2 * DF), U32),
            pltpu.VMEM((HP, D // 2, LANES), U32),
            pltpu.VMEM((HP, LANES // 2, DF), U32),
            pltpu.VMEM((NB + 1, LANES, DP), F32),
            pltpu.VMEM((NB + 1, LANES, DP), F32),
            pltpu.VMEM((NB, D, LANES), F32),
            pltpu.VMEM((D, LANES), BF16),
            pltpu.VMEM((D, F), F32),
            pltpu.VMEM((D, S), A_x.dtype),
            pltpu.VMEM((D, F), BF16),
            pltpu.VMEM((1, S), F32),
            pltpu.SemaphoreType.DMA((4, HP)),
            pltpu.SemaphoreType.DMA((NB,)),
            pltpu.SemaphoreType.DMA((NB,)),
            pltpu.SemaphoreType.DMA((1,)),
            pltpu.SemaphoreType.DMA((S // TB,)),
        ],
        compiler_params=pltpu.CompilerParams(vmem_limit_bytes=110 * 2**20),
    )(
        jnp.swapaxes(A_x, 1, 2).reshape(D, S),
        A_mem0.reshape(M, D),
        hc(A_Wq), hc(A_Wk), hc(A_Wv),
        jnp.swapaxes(A_Wo, 1, 2),
        B_w1, B_b1, B_w2, B_b2,
    )
    return jnp.swapaxes(outT.reshape(B, D, S), 1, 2)
```

```python
import functools

import jax
import jax.numpy as jnp
from jax import lax
import jax.experimental.pallas as pl
import jax.experimental.pallas.tpu as pltpu

LANES = 128
SUB = 8
EPS = 1e-5
NEG = -1000000000.0
F32 = jnp.float32
BF16 = jnp.bfloat16
U32 = jnp.uint32

PRODUCTS = (
    (((1, -1, 0), (0, 0, 0), (-1, 0, 0)), ((1, 0, 0), (0, 0, 0)), ((1, 0, 0), (-1, 0, 0)),
     0, ((1, 0, 0), (1, 0, 0)), None),
    (((1, 0, -1), (-1, 0, 0), (0, 0, 0)), ((1, 0, 0), (1, 0, 0)), ((0, 0, 0), (1, 0, 0)),
     1, None, ((1, 0, 0), (1, 0, 0))),
    (((0, 0, 0), (-1, 1, 0), (0, -1, 0)), ((0, 1, 0), (0, 0, 0)), ((0, 1, 0), (0, 0, 0)),
     0, ((0, 1, 0), (0, 1, 0)), None),
    (((0, -1, 0), (0, 1, 1), (0, 0, 0)), ((0, 0, 0), (0, 1, 0)), ((0, 0, 0), (0, 1, 0)),
     1, None, ((0, 1, 0), (0, 1, 0))),
    (((0, 0, 0), (0, 0, -1), (-1, 0, 1)), ((0, 0, 1), (0, 0, 1)), ((0, 0, 1), (0, 0, 0)),
     0, ((0, 0, 1), (0, 0, 1)), None),
    (((0, 0, 1), (0, 0, 0), (0, -1, -1)), ((0, 0, 0), (0, 0, 1)), ((0, 0, 1), (0, 0, -1)),
     1, None, ((0, 0, 1), (0, 0, -1))),
    (((0, 0, 0), (1, 0, 0), (0, 0, 0)), ((1, 1, 0), (1, 1, 0)), ((1, 1, 0), (0, 0, 0)),
     0, ((1, 1, 0), (1, 1, 0)), ((1, 1, 0), (1, 0, 0))),
    (((0, 1, 0), (-1, 0, 0), (0, 0, 0)), ((1, 0, 0), (1, 1, 0)), ((1, 1, 0), (-1, 0, 0)),
     0, ((1, 0, 0), (1, 1, 0)), None),
    (((0, 1, 0), (0, 0, 0), (0, 0, 0)), ((0, 0, 0), (1, 1, 0)), ((-1, -1, 0), (1, 1, 0)),
     1, None, ((1, 1, 0), (0, 1, 0))),
    (((0, 0, 0), (0, 0, 1), (0, 0, 0)), ((0, 1, 1), (0, 1, 1)), ((0, 0, 0), (0, -1, 1)),
     1, ((0, 1, 1), (0, 0, 1)), ((0, 1, 1), (0, -1, 1))),
    (((0, 0, 0), (0, 0, 1), (0, 1, 0)), ((0, 1, 1), (0, 0, 1)), ((0, 0, 1), (0, 1, -1)),
     1, None, ((0, 0, 1), (0, 1, -1))),
    (((0, 0, 0), (0, 0, 0), (0, 1, 0)), ((0, 1, 1), (0, 0, 0)), ((0, 1, -1), (0, -1, 1)),
     0, ((0, 1, 1), (0, 1, 0)), None),
    (((0, 0, 1), (0, 0, 0), (-1, 0, 0)), ((1, 0, 0), (0, 0, -1)), ((0, 0, 1), (1, 0, 0)),
     0, ((1, 0, 0), (0, 0, 1)), ((0, 0, 1), (-1, 0, 0))),
    (((0, 0, 1), (0, 0, 0), (0, 0, 0)), ((0, 0, 0), (1, 0, 1)), ((0, 0, 0), (1, 0, 1)),
     1, None, ((1, 0, 1), (1, 0, 1))),
    (((0, 0, 0), (0, 0, 0), (1, 0, 0)), ((1, 0, 1), (0, 0, 0)), ((1, 0, 1), (0, 0, 0)),
     0, ((1, 0, 1), (1, 0, 1)), None),
)
EARLY = tuple(r for r, prod in enumerate(PRODUCTS) if prod[3] == 1 and any(prod[2][0]))

PASS_ORDER = ((11, 7, 6, 14, 0, 2, 9, 4, 12), (1, 8, 3, 13, 9, 5, 6, 12, 10))
STEP_ORDER = (
    'k0 k1 k2 k3 ks v0 v1 r v2 s v3 vs u0 u1 o0 o1 px o2 b2 os u2 u3'.split(),
    'k0 k1 k2 k3 ks v0 v1 r v2 s v3 vs u0 u1 os o0 o1 px o2 b2 u2 u3'.split(),
)
MIX_PIECES = 4
NEXT_X_AT = 6
OUT_UNROLL = 3


def _dot(a, b):
    return jnp.dot(a, b, preferred_element_type=F32)


def _dot_nt(a, b):
    return lax.dot_general(a, b, (((1,), (1,)), ((), ())), preferred_element_type=F32)


def _dot_split(a, b, parts):
    n = a.shape[0] // parts
    return jnp.concatenate([_dot(a[i * n:(i + 1) * n], b) for i in range(parts)], axis=0)


def _pack(x):
    return pltpu.bitcast(x.astype(BF16), U32)


def _unpack(w):
    return pltpu.bitcast(w, BF16)


def _split_words(words):
    low = lax.bitcast_convert_type(words << 16, F32)
    high = lax.bitcast_convert_type(words & jnp.uint32(0xFFFF0000), F32)
    return low, high


def _tree(op, terms):
    while len(terms) > 1:
        terms = [op(terms[i], terms[i + 1]) if i + 1 < len(terms) else terms[i]
                 for i in range(0, len(terms), 2)]
    return terms[0]


def _combine(terms):
    sign, total = 0, None
    for c, v in terms:
        if not c:
            continue
        if total is None:
            sign, total = c, v
        elif c == sign:
            total = total + v
        elif sign > 0:
            total = total - v
        else:
            sign, total = c, v - total
    return total if sign > 0 else -total


def _layernorm(x, n):
    full = n // LANES * LANES
    lane = lax.broadcasted_iota(jnp.int32, (x.shape[0], LANES), 1)

    def mean(v):
        tiles = [v[:, c:c + LANES] for c in range(0, full, LANES)]
        tiles.append(jnp.where(lane < n - full, v[:, full:], 0.0))
        return jnp.sum(_tree(jnp.add, tiles), axis=1, keepdims=True) * (1.0 / n)

    xc = x - mean(x)
    return xc * lax.rsqrt(mean(xc * xc) + EPS)


def _gelu(u):
    c = 0.7978845608028654
    half = 0.5 * u
    return half * jnp.tanh(u * (c + (c * 0.044715) * (u * u))) + half


def _group_allreduce(x, op, lane):
    pos = lane & (SUB - 1)
    return _tree(op, [x] + [jnp.where(pos >= j, pltpu.roll(x, j, 1), pltpu.roll(x, LANES - SUB + j, 1))
                            for j in range(1, SUB)])


def _barrel(vs, lane, blk):
    n = len(vs)
    sh = 1
    while sh < n:
        high = (lane & (blk * sh)) != 0
        nxt = []
        for r in range(n):
            a, b = vs[r], vs[(r + sh) % n]
            nxt.append(b if a is None else a if b is None else jnp.where(high, b, a))
        vs = nxt
        sh *= 2
    return vs


def _strassen_lhs(a11, a12, a21, a22):
    return [a11 + a22, a21 + a22, a11, a22, a11 + a12, a21 - a11, a12 - a22]


def _strassen_rhs(b11, b12, b21, b22):
    f11, f12, f21, f22 = (b.astype(F32) for b in (b11, b12, b21, b22))
    return [v.astype(BF16) for v in (f11 + f22, f11, f12 - f22, f21 - f11, f22, f11 + f12, f21 + f22)]


def _strassen_sum(m1, m2, m3, m4, m5, m6, m7):
    return (m1 + m7) + (m4 - m5), m3 + m5, m2 + m4, (m1 + m6) + (m3 - m2)


def _kernel(xT_hbm, mem0_hbm, wq_hbm, wk_hbm, wv_hbm, woT_hbm, w1_hbm, b1_hbm, w2_hbm, b2_hbm,
            outT_hbm,
            wq_s, wk_s, wv_s, wo_s, xT_s, w1_s, w2_s, mem0_s, b1_raw, b2_raw,
            w_main, w_rest, w_qrest, w_krest, w_vrest, w_orest, early_s, early_rest_s, xn_s,
            x_s, h_s, hn_s, hnT_s, lhs_s, u_s, g_s, b2_s, out_s,
            small_sem, w_sem, x_sem, w1_sem, w2_sem, out_sem, *, seg, scale):
    NP, D, TP = xT_s.shape
    S = NP * TP
    HP = w_orest.shape[0]
    M = mem0_s.shape[0]
    L = M + seg
    F = u_s.shape[1]
    DF = D // LANES * LANES
    DR = D - DF
    NT = DF // LANES
    KG = L // SUB
    SPP = TP // seg
    DH, FH = D // 2, F // 2
    d0, d1 = slice(0, LANES), slice(LANES, 2 * LANES)

    def offset(i, n):
        return i * n if isinstance(i, int) else pl.multiple_of(i * n, n)

    def pair_copy(i, src, dst, hp):
        return pltpu.make_async_copy(src.bitcast(U32).at[:, hp, :], dst.at[hp], w_sem.at[i * HP + hp])

    def qk_copies(hp):
        return [pair_copy(0, wk_hbm, wk_s, hp), pair_copy(1, wq_hbm, wq_s, hp)]

    def vo_copies(hp):
        two = pl.ds(2 * hp, 2)
        return [pair_copy(2, wv_hbm, wv_s, hp),
                pltpu.make_async_copy(woT_hbm.at[two], wo_s.at[two], w_sem.at[3 * HP + hp])]

    def x_copy(p):
        return pltpu.make_async_copy(xT_hbm.at[:, pl.ds(offset(p, TP), TP)], xT_s.at[p], x_sem.at[p])

    def w1_copy(p):
        return pltpu.make_async_copy(w1_hbm.at[pl.ds(offset(p, TP), TP)], w1_s.at[p], w1_sem.at[p])

    def out_copy(p):
        cols = pl.ds(offset(p, TP), TP)
        return pltpu.make_async_copy(out_s.at[:, cols], outT_hbm.at[:, cols], out_sem.at[p])

    w2_copy = pltpu.make_async_copy(w2_hbm, w2_s, w2_sem.at[0])
    small_copies = [pltpu.make_async_copy(src, dst, small_sem.at[i]) for i, (src, dst) in enumerate(
        ((mem0_hbm, mem0_s), (b1_hbm, b1_raw), (b2_hbm, b2_raw)))] + [x_copy(0)]
    for cp in small_copies:
        cp.start()

    def start_qk(hp, c):
        for cp in qk_copies(hp):
            cp.start()
        return c

    lax.fori_loop(0, HP, start_qk, 0)

    def fuse_pair(l0, l1, r0, r1):
        cols = jnp.concatenate([_dot_nt(r0[DF:], l0), _dot_nt(r1[DF:], l1)], axis=0)
        cols = jnp.concatenate([cols, jnp.zeros((LANES, LANES - DR), F32)], axis=1).T[:D]
        a0, a1 = (_dot_nt(jnp.concatenate([l[DF:], l[:DF]], axis=0), r[:DF]) for l, r in ((l0, r0), (l1, r1)))
        return a0[DR:], a1[DR:], cols, jnp.concatenate([a0[:DR], a1[:DR]], axis=0)

    def store_main(unit, a):
        for r, prod in enumerate(PRODUCTS):
            w_main[r, unit] = _pack(_combine(
                [(prod[0][k][n], a[k * LANES:(k + 1) * LANES, n * LANES:(n + 1) * LANES])
                 for k in range(NT) for n in range(NT)]))

    def qk_body(hp, c):
        for cp in qk_copies(hp):
            cp.wait()
        for cp in vo_copies(hp):
            cp.start()
        q0, q1 = _split_words(wq_s[hp])
        k0, k1 = _split_words(wk_s[hp])
        a0, a1, cols, rows = fuse_pair(k0 * scale, k1 * scale, q0, q1)
        store_main(2 * hp, a0)
        store_main(2 * hp + 1, a1)
        rows = rows.T
        for i, w in enumerate(_strassen_rhs(rows[d0], cols[d0], rows[d1], cols[d1])):
            w_rest[i, hp] = pltpu.bitcast(w, U32)
        w_qrest[hp] = _pack(rows[2 * LANES:])
        w_krest[hp] = _pack(cols[2 * LANES:])
        return c

    def vo_body(hp, c):
        for cp in vo_copies(hp):
            cp.wait()
        v0, v1 = _split_words(wv_s[hp])
        a0, a1, cols, rows = fuse_pair(v0, v1, wo_s[2 * hp], wo_s[2 * hp + 1])
        store_main(2 * (HP + hp), a0)
        store_main(2 * (HP + hp) + 1, a1)
        w_vrest[hp] = _pack(cols)
        w_orest[hp] = _pack(rows)
        return c

    def x_rows(p):
        for c in range(0, TP, LANES):
            xT = xT_s[p, :, c:c + LANES].astype(F32)
            x_s[p, c:c + LANES, :] = jnp.concatenate([xT, xT[DF:]], axis=0).T

    def x_pair(p, j):
        return [_layernorm(x_s[p, (j + k) * seg:(j + k + 1) * seg, :], D) for k in range(2)]

    hn_s[0] = jnp.zeros(hn_s.shape[1:], F32)
    h_s[0, TP - seg:, :] = jnp.zeros((seg, h_s.shape[2]), F32)
    for cp in small_copies:
        cp.wait()
    x_rows(0)
    xn_s[0], xn_s[1] = x_pair(0, 0)
    u_s[...] = jnp.broadcast_to(b1_raw[...].astype(F32).reshape(1, F), u_s.shape)
    b2_s[...] = b2_raw[...].astype(F32).reshape(1, S)
    lax.fori_loop(0, HP, qk_body, 0)
    x_copy(1).start()
    w1_copy(0).start()
    lax.fori_loop(0, HP, vo_body, 0)
    for p in range(1, NP):
        if p + 1 < NP:
            x_copy(p + 1).start()
        w1_copy(p).start()
    w2_copy.start()

    def all_pairs(ref):
        return _unpack(jnp.concatenate([ref[p] for p in range(HP)], axis=1))

    def main_weights(r, pair):
        return _unpack(jnp.concatenate([w_main[r, 2 * pair], w_main[r, 2 * pair + 1]], axis=1))

    def token_operand(r, xa, xb):
        return _combine([(PRODUCTS[r][1][i][k], x[:, k * LANES:(k + 1) * LANES])
                         for i, x in enumerate((xa, xb)) for k in range(NT)])

    def main_projection(step, mem, now, ahead, saved):
        lhs = {}
        for r, prod in enumerate(PRODUCTS):
            rows = []
            if prod[4 + step] is not None:
                rows.append(_combine([(c, mem[:, k * LANES:(k + 1) * LANES])
                                      for k, c in enumerate(prod[4 + step][0])]))
            if prod[3] == step:
                rows.append(token_operand(r, *(ahead if r in EARLY else now)))
            if rows:
                lhs[r] = jnp.concatenate(rows, axis=0)

        def project(pair):
            prods = {r: _dot(lhs[r], main_weights(r, pair)) for r in PASS_ORDER[step]}
            mem_rows = [_combine([(PRODUCTS[r][4 + step][1][n], v[:M]) for r, v in prods.items()
                                  if PRODUCTS[r][4 + step] is not None]) for n in range(NT)]
            tok = {r: v[-seg:] for r, v in prods.items() if PRODUCTS[r][3] == step}
            if step == 0:
                tok = {**dict(zip(EARLY, saved[pair])), **tok}
                out, saved[pair] = ([_combine([(PRODUCTS[r][2][i][n], v) for r, v in tok.items()])
                                     for n in range(NT)] for i in range(2))
            else:
                out = [_combine([(1, saved[pair][n])] + [(PRODUCTS[r][2][1][n], v) for r, v in tok.items()
                                                         if r not in EARLY]) for n in range(NT)]
                saved[pair] = [tok[r] for r in EARLY]
            full = [jnp.concatenate([m, x], axis=0) for m, x in zip(mem_rows, out)]
            return [[f[:, h * LANES:(h + 1) * LANES] for f in full] for h in range(2)]
        return project

    half = seg // 2

    def rest_dot(m, x, i):
        return _dot(jnp.concatenate([m, x], axis=0), all_pairs(w_rest.at[i]))

    def rest_ahead(xa, xb):
        return xa[:, d1] - xb[:, d1], (xa[:, d0] + xa[:, d1])[half:]

    def rest_projection(step, mem, now, ahead, saved):
        m1, m2 = mem[:, d0], mem[:, d1]
        xa, xb = now

        def project():
            if step == 0:
                p7, p5_rest = saved['rest']
                p1 = rest_dot(m1 + m2, xa[:, d0] + xb[:, d1], 0)
                p3 = rest_dot(m1, xa[:, d0], 2)
                p5 = jnp.concatenate([rest_dot(m1 + m2, (xa[:, d0] + xa[:, d1])[:half], 4), p5_rest], axis=0)
                p4 = rest_dot(m2, xb[:, d1], 3)
                saved['rest'] = (p4[M:], p1[M:] + p3[M:])
                n1 = (p1 + p4) - p5
                return jnp.concatenate([n1[:M], n1[M:] + p7], axis=0), p3 + p5
            t1, t2 = saved['rest']
            x7, x5 = rest_ahead(*ahead)
            p2 = rest_dot(m1, xb[:, d0] + xb[:, d1], 1)
            p6 = rest_dot(m1, xb[:, d0] - xa[:, d0], 5)
            p5 = rest_dot(m2, x5, 4)
            p7 = rest_dot(m2, x7, 6)
            saved['rest'] = (p7[M:], p5[M:])
            return (p2 + jnp.concatenate([p7[:M] - p5[:M], t1], axis=0),
                    (p6 - p2) + jnp.concatenate([p5[:M], t2], axis=0))
        return project

    def segment(order, xs, mem, project, project_rest, filler, neg):
        row = lax.broadcasted_iota(jnp.int32, (L, LANES), 0)
        lane = lax.broadcasted_iota(jnp.int32, (L, LANES), 1)
        low = lane < DR
        blk = 2 * SUB
        hs = jnp.concatenate([mem, xs], axis=0)
        res = {}

        def stack(heads):
            return jnp.concatenate([h[g * SUB:(g + 1) * SUB] for g in range(KG) for h in heads], axis=0)

        def main_tile(kind, t):
            return [head[t] for i in range(HP // 2) for head in res[kind + str(i)]]

        def by_head(shared):
            out = []
            for p in range(HP):
                t = shared[:, p * LANES:(p + 1) * LANES]
                out += [jnp.where(low, t, 0.0), jnp.where(low, 0.0, t)]
            return out

        first, second = jnp.where(low, hs[:, DF:], 0.0), jnp.where(low, 0.0, hs[:, DF:])
        keys = [jnp.concatenate([first[g * SUB:(g + 1) * SUB], second[g * SUB:(g + 1) * SUB]], axis=0)
                for g in range(KG)] + [jnp.zeros((blk, LANES), F32)] * (HP - KG)

        def scores_rest():
            q = jnp.concatenate([res['q'][:, p * LANES:(p + 1) * LANES] for p in range(HP)], axis=0)
            r = _dot(q, jnp.concatenate(keys, axis=0).T.astype(BF16))
            r = [r[p * L:(p + 1) * L] for p in range(HP)]
            r = _barrel([pltpu.roll(t, blk * p, 1) if p else t for p, t in enumerate(r)], lane, blk)
            return [pltpu.roll(r[-g % HP], LANES - blk * g, 1) if g else r[0] for g in range(KG)]

        def scores_main():
            k = jnp.concatenate([stack(main_tile('k', t)) for t in range(NT)] + [stack(by_head(res['ks']))],
                                axis=1)
            out = []
            for g in range(KG):
                begin = max(M, g * SUB)
                t = _dot(jnp.concatenate([hs[:M], hs[begin:]], axis=0),
                         k[g * LANES:(g + 1) * LANES].T.astype(BF16))
                gap = [jnp.zeros((begin - M, LANES), F32)] if begin > M else []
                out.append(jnp.concatenate([t[:M]] + gap + [t[M:]], axis=0))
            return out

        def softmax():
            if 'p' not in res:
                tiles = []
                for g in range(KG):
                    key = g * SUB + (lane & (SUB - 1))
                    tiles.append(jnp.where((row < M) | (row >= key), res['s'][g] + res['r'][g], neg))
                top = _group_allreduce(functools.reduce(jnp.maximum, tiles), jnp.maximum, lane)
                ex = [jnp.exp(t - top) for t in tiles]
                inv = 1.0 / _group_allreduce(functools.reduce(jnp.add, ex), jnp.add, lane)
                res['p'] = [e * inv for e in ex]
            return res['p']

        def mix_rest():
            p = [pltpu.roll(t, blk * g, 1) if g else t for g, t in enumerate(softmax())]
            p = _barrel(p + [None] * (HP - KG), lane, blk)
            return jnp.concatenate(
                [_dot(p[-i % HP], jnp.concatenate([keys[(j - i) % HP] for j in range(HP)], axis=0).astype(BF16))
                 for i in range(HP)], axis=1)

        def mix(values):
            return _dot(jnp.concatenate(softmax(), axis=1), stack(values).astype(BF16))

        for name in order:
            if name == 'ks':
                q, k = project_rest()
                res['ks'] = k + _dot(hs[:, 2 * LANES:D], all_pairs(w_krest))
                res['q'] = q + _dot(hs[:, 2 * LANES:DF], all_pairs(w_qrest))
            elif name == 'vs':
                res[name] = _dot(hs[:, :D], all_pairs(w_vrest))
            elif name[0] in 'kv':
                pair = HP * (name[0] == 'v') + 2 * int(name[1])
                res[name] = project(pair) + project(pair + 1)
            elif name == 'r':
                res[name] = scores_rest()
            elif name == 's':
                res[name] = scores_main()
            elif name == 'px':
                res[name] = mix_rest()
            elif name == 'b2':
                res[name] = _dot(res['px'], _unpack(jnp.concatenate([w_orest[p] for p in range(HP)], axis=0)))
            elif name == 'os':
                res[name] = mix(by_head(res['vs']))
            elif name[0] == 'o':
                res[name] = mix(main_tile('v', int(name[1])))
            else:
                filler(int(name[1]))
        o = jnp.concatenate([res['o%d' % t] for t in range(NT)], axis=1) + res['b2']
        o = jnp.concatenate([o, res['os'] + pltpu.roll(res['os'], DR, 1)], axis=1)
        return o[:M], o[M:]

    def mixer_norm(h):
        return _layernorm(_layernorm(h, D), D)

    def transpose_hn(slot, c):
        hnT_s[:, c:c + LANES] = hn_s[slot, c:c + LANES, :].T[:D]

    def mixer_operands():
        ops = _strassen_lhs(hnT_s[:DH, d0], hnT_s[:DH, d1], hnT_s[DH:, d0], hnT_s[DH:, d1])
        for i, a in enumerate(ops):
            lhs_s[i] = a

    def hidden_cols(t):
        return slice(t * LANES, (t + 1) * LANES), slice(FH + t * LANES, FH + (t + 1) * LANES)

    def w1_operands(p, c1, c2):
        return _strassen_rhs(w1_s[p, d0, c1], w1_s[p, d0, c2], w1_s[p, d1, c1], w1_s[p, d1, c2])

    def accumulate(p, t, piece):
        c1, c2 = hidden_cols(t)
        rhs = w1_operands(p, c1, c2)
        n = DH // MIX_PIECES
        top, bot = slice(piece * n, (piece + 1) * n), slice(DH + piece * n, DH + (piece + 1) * n)
        c11, c12, c21, c22 = _strassen_sum(*[_dot(lhs_s[i, top], rhs[i]) for i in range(7)])
        u_s[top, c1] += c11
        u_s[top, c2] += c12
        u_s[bot, c1] += c21
        u_s[bot, c2] += c22

    def pair_cols(pair):
        return slice(2 * pair * LANES, 2 * (pair + 1) * LANES)

    def pair_body(p, mem):
        w1_copy(p).wait()

        @pl.when(p + 1 < NP)
        def _():
            x_copy(p + 1).wait()

        prev, following = jnp.maximum(p - 1, 0), jnp.minimum(p + 1, NP - 1)
        zero = jnp.minimum(p, 0)

        def mask_value_after(*refs):
            neg = jnp.full((SUB, LANES), NEG, F32)
            for ref in refs:
                neg = jnp.where(p < 0, ref[zero, :SUB, :LANES], neg)
            return jnp.concatenate([neg] * KG, axis=0)

        saved = {pair: [early_s[i, :, pair_cols(pair)] for i in range(len(EARLY))] for pair in range(2 * HP)}
        saved['rest'] = (early_rest_s[:seg], early_rest_s[seg:])
        now = xn_s[0], xn_s[1]
        for j in range(SPP):
            rows = slice(j * seg, (j + 1) * seg)
            x = x_s[p, rows, :]
            pins = [hn_s]
            if j == 0:
                hn_s[p, TP - seg:, :] = mixer_norm(h_s[p, TP - seg:, :])
                for c in range(0, TP, LANES):
                    transpose_hn(p, c)
                mixer_operands()
            else:
                hn_s[p + 1, (j - 1) * seg:j * seg, :] = mixer_norm(h)
            if j == NEXT_X_AT:
                x_rows(following)
                pins.append(x_s)
            step, tile = j % 2, j - (SPP - FH // LANES)
            ahead = None
            if step:
                ahead = x_pair(p, j + 1) if j + 1 < SPP else x_pair(following, 0)
            args = (step, mem, now, ahead, saved)
            mem, att = segment(STEP_ORDER[step], now[step], mem, main_projection(*args), rest_projection(*args),
                               functools.partial(accumulate, prev, tile) if tile >= 0 else lambda piece: None,
                               mask_value_after(*pins))
            if step:
                now = ahead
            h = x + att
            h_s[p + 1, rows, :] = h
        xn_s[0], xn_s[1] = now
        early_rest_s[:seg], early_rest_s[seg:] = saved['rest']
        for pair in range(2 * HP):
            for i, v in enumerate(saved[pair]):
                early_s[i, :, pair_cols(pair)] = v
        return mem

    start = xn_s[0], xn_s[1]
    x7, x5 = rest_ahead(*start)
    early_rest_s[:seg], early_rest_s[seg:] = _dot(x7, all_pairs(w_rest.at[6])), _dot(x5, all_pairs(w_rest.at[4]))
    for i, r in enumerate(EARLY):
        for pair in range(2 * HP):
            early_s[i, :, pair_cols(pair)] = _dot(token_operand(r, *start), main_weights(r, pair))
    mem0 = mem0_s[...].astype(F32)
    lax.fori_loop(0, NP, pair_body, jnp.concatenate([mem0, mem0[:, DF:]], axis=1))

    def out_cols(p):
        return pl.ds(offset(2 * p, LANES), LANES), pl.ds(offset(2 * p + 1, LANES), LANES)

    def w2_operands(p, k1, k2):
        n1, n2 = out_cols(p)
        return _strassen_rhs(w2_s[k1, n1], w2_s[k1, n2], w2_s[k2, n1], w2_s[k2, n2])

    def out_store(p, c11, c12, c21, c22):
        for k, (cols, top, bot) in enumerate(zip(out_cols(p), (c11, c12), (c21, c22))):
            h = h_s[p + 1, k * LANES:(k + 1) * LANES, :].T[:D]
            y = jnp.concatenate([top, bot], axis=0)
            out_s[:, cols] = (h + (y + b2_s[:, cols])).astype(out_s.dtype)
        out_copy(p).start()

    def out_block(p):
        rhs = w2_operands(p, slice(0, FH), slice(FH, F))
        out_store(p, *_strassen_sum(*[_dot(g_s[i], rhs[i]) for i in range(7)]))

    w2_copy.wait()
    tiles = [hidden_cols(t) for t in range(FH // LANES)]
    transpose_hn(NP, 0)
    x11, x21 = hnT_s[:DH, d0], hnT_s[DH:, d0]
    for c1, c2 in tiles:
        rhs = w1_operands(NP - 1, c1, c2)
        m3, m6 = _dot_split(x11, rhs[2], 2), _dot_split(x21 - x11, rhs[5], 2)
        u_s[:DH, c2] += m3
        u_s[DH:, c2] += m3 + m6
    hn_s[NP, TP - seg:, :] = mixer_norm(h_s[NP, TP - seg:, :])
    transpose_hn(NP, LANES)
    mixer_operands()

    acc, ready = None, []

    def drain(acc):
        k1 = slice(ready[0][1].start, ready[-1][1].stop)
        k2 = slice(ready[0][2].start, ready[-1][2].stop)
        lhs = [jnp.concatenate([r[0][i] for r in ready], axis=1) for i in range(7)]
        prods = [_dot_split(a, b, 2) for a, b in zip(lhs, w2_operands(0, k1, k2))]
        ready.clear()
        return prods if acc is None else [a + b for a, b in zip(acc, prods)]

    for t, (c1, c2) in enumerate(tiles):
        rhs = w1_operands(NP - 1, c1, c2)
        m1, m2, m4, m5, m7 = (_dot_split(lhs_s[i], rhs[i], MIX_PIECES) for i in (0, 1, 3, 4, 6))
        if t and t % 2 == 0:
            acc = drain(acc)
        ops = _strassen_lhs(_gelu(u_s[:DH, c1] + ((m1 + m7) + (m4 - m5))), _gelu(u_s[:DH, c2] + m5),
                            _gelu(u_s[DH:, c1] + (m2 + m4)), _gelu(u_s[DH:, c2] + (m1 - m2)))
        for i, a in enumerate(ops):
            g_s[i, :, c1] = a
        ready.append((ops, c1, c2))
    out_store(0, *_strassen_sum(*drain(acc)))
    peeled = 1 + (NP - 1) % OUT_UNROLL
    for p in range(1, peeled):
        out_block(p)

    def out_body(i, c):
        for k in range(OUT_UNROLL):
            out_block(peeled + i * OUT_UNROLL + k)
        return c

    if NP > peeled:
        lax.fori_loop(0, (NP - peeled) // OUT_UNROLL, out_body, 0)
    for p in range(NP):
        out_copy(p).wait()


@functools.partial(jax.jit, static_argnames=("A_seg_len",))
def pallas_sequential_preLN__memory_aug_recurrent_mem_tr__mixer_token_mlp__prompt_kernel(
        A_x, A_mem0, A_Wq, A_Wk, A_Wv, A_Wo, A_seg_len, B_x, B_w1, B_b1, B_w2, B_b2):
    del B_x
    B, S, D = A_x.shape
    _, H, E = A_Wq.shape
    M = A_mem0.shape[1]
    F = B_w1.shape[1]
    seg = int(A_seg_len)
    HP = H // 2
    DF = D // LANES * LANES
    DP = DF + LANES
    TP = 2 * LANES
    NP = S // TP
    assert B == 1 and M == SUB and seg == 4 * SUB and H * SUB == LANES
    assert DF == 3 * LANES and 2 * (D - DF) == LANES and S % TP == 0 and F == 7 * TP
    hbm = pl.BlockSpec(memory_space=pl.ANY)
    outT = pl.pallas_call(
        functools.partial(_kernel, seg=seg, scale=E ** -0.5),
        out_shape=jax.ShapeDtypeStruct((D, S), A_x.dtype),
        in_specs=[hbm] * 10,
        out_specs=hbm,
        scratch_shapes=[
            pltpu.VMEM((HP, D, E), U32),
            pltpu.VMEM((HP, D, E), U32),
            pltpu.VMEM((HP, D, E), U32),
            pltpu.VMEM((H, D, E), BF16),
            pltpu.VMEM((NP, D, TP), BF16),
            pltpu.VMEM((NP, TP, F), BF16),
            pltpu.VMEM((F, S), BF16),
            pltpu.VMEM((M, D), BF16),
            pltpu.VMEM((F,), BF16),
            pltpu.VMEM((S,), BF16),
            pltpu.VMEM((len(PRODUCTS), 2 * H, LANES // 2, LANES), U32),
            pltpu.VMEM((7, HP, LANES // 2, LANES), U32),
            pltpu.VMEM((HP, LANES // 2, LANES), U32),
            pltpu.VMEM((HP, (D - 2 * LANES) // 2, LANES), U32),
            pltpu.VMEM((HP, D // 2, LANES), U32),
            pltpu.VMEM((HP, LANES // 2, DF), U32),
            pltpu.VMEM((len(EARLY), seg, 2 * H * LANES), F32),
            pltpu.VMEM((seg + seg // 2, HP * LANES), F32),
            pltpu.VMEM((2, seg, DP), F32),
            pltpu.VMEM((NP, TP, DP), F32),
            pltpu.VMEM((NP + 1, TP, DP), F32),
            pltpu.VMEM((NP + 1, TP, DP), F32),
            pltpu.VMEM((D, TP), F32),
            pltpu.VMEM((7, D // 2, LANES), F32),
            pltpu.VMEM((D, F), F32),
            pltpu.VMEM((7, D // 2, F // 2), F32),
            pltpu.VMEM((1, S), F32),
            pltpu.VMEM((D, S), A_x.dtype),
            pltpu.SemaphoreType.DMA((3,)),
            pltpu.SemaphoreType.DMA((4 * HP,)),
            pltpu.SemaphoreType.DMA((NP,)),
            pltpu.SemaphoreType.DMA((NP,)),
            pltpu.SemaphoreType.DMA((1,)),
            pltpu.SemaphoreType.DMA((NP,)),
        ],
        compiler_params=pltpu.CompilerParams(vmem_limit_bytes=110 * 2**20),
    )(
        jnp.swapaxes(A_x, 1, 2).reshape(D, S),
        A_mem0.reshape(M, D),
        A_Wq, A_Wk, A_Wv,
        jnp.swapaxes(A_Wo, 1, 2),
        B_w1, B_b1, B_w2, B_b2,
    )
    return jnp.swapaxes(outT.reshape(B, D, S), 1, 2)
```

```python
import functools

import jax
import jax.numpy as jnp
from jax import lax
import jax.experimental.pallas as pl
import jax.experimental.pallas.tpu as pltpu

LANES = 128
SUB = 8
EPS = 1e-5
NEG = -1000000000.0
F32 = jnp.float32
BF16 = jnp.bfloat16
U32 = jnp.uint32

PRODUCTS = (
    (((1, -1, 0), (0, 0, 0), (-1, 0, 0)), ((1, 0, 0), (0, 0, 0)), ((1, 0, 0), (-1, 0, 0)),
     0, ((1, 0, 0), (1, 0, 0)), None),
    (((1, 0, -1), (-1, 0, 0), (0, 0, 0)), ((1, 0, 0), (1, 0, 0)), ((0, 0, 0), (1, 0, 0)),
     1, None, ((1, 0, 0), (1, 0, 0))),
    (((0, 0, 0), (-1, 1, 0), (0, -1, 0)), ((0, 1, 0), (0, 0, 0)), ((0, 1, 0), (0, 0, 0)),
     0, ((0, 1, 0), (0, 1, 0)), None),
    (((0, -1, 0), (0, 1, 1), (0, 0, 0)), ((0, 0, 0), (0, 1, 0)), ((0, 0, 0), (0, 1, 0)),
     1, None, ((0, 1, 0), (0, 1, 0))),
    (((0, 0, 0), (0, 0, -1), (-1, 0, 1)), ((0, 0, 1), (0, 0, 1)), ((0, 0, 1), (0, 0, 0)),
     0, ((0, 0, 1), (0, 0, 1)), None),
    (((0, 0, 1), (0, 0, 0), (0, -1, -1)), ((0, 0, 0), (0, 0, 1)), ((0, 0, 1), (0, 0, -1)),
     1, None, ((0, 0, 1), (0, 0, -1))),
    (((0, 0, 0), (1, 0, 0), (0, 0, 0)), ((1, 1, 0), (1, 1, 0)), ((1, 1, 0), (0, 0, 0)),
     0, ((1, 1, 0), (1, 1, 0)), ((1, 1, 0), (1, 0, 0))),
    (((0, 1, 0), (-1, 0, 0), (0, 0, 0)), ((1, 0, 0), (1, 1, 0)), ((1, 1, 0), (-1, 0, 0)),
     0, ((1, 0, 0), (1, 1, 0)), None),
    (((0, 1, 0), (0, 0, 0), (0, 0, 0)), ((0, 0, 0), (1, 1, 0)), ((-1, -1, 0), (1, 1, 0)),
     1, None, ((1, 1, 0), (0, 1, 0))),
    (((0, 0, 0), (0, 0, 1), (0, 0, 0)), ((0, 1, 1), (0, 1, 1)), ((0, 0, 0), (0, -1, 1)),
     1, ((0, 1, 1), (0, 0, 1)), ((0, 1, 1), (0, -1, 1))),
    (((0, 0, 0), (0, 0, 1), (0, 1, 0)), ((0, 1, 1), (0, 0, 1)), ((0, 0, 1), (0, 1, -1)),
     1, None, ((0, 0, 1), (0, 1, -1))),
    (((0, 0, 0), (0, 0, 0), (0, 1, 0)), ((0, 1, 1), (0, 0, 0)), ((0, 1, -1), (0, -1, 1)),
     0, ((0, 1, 1), (0, 1, 0)), None),
    (((0, 0, 1), (0, 0, 0), (-1, 0, 0)), ((1, 0, 0), (0, 0, -1)), ((0, 0, 1), (1, 0, 0)),
     0, ((1, 0, 0), (0, 0, 1)), ((0, 0, 1), (-1, 0, 0))),
    (((0, 0, 1), (0, 0, 0), (0, 0, 0)), ((0, 0, 0), (1, 0, 1)), ((0, 0, 0), (1, 0, 1)),
     1, None, ((1, 0, 1), (1, 0, 1))),
    (((0, 0, 0), (0, 0, 0), (1, 0, 0)), ((1, 0, 1), (0, 0, 0)), ((1, 0, 1), (0, 0, 0)),
     0, ((1, 0, 1), (1, 0, 1)), None),
)
EARLY = tuple(r for r, prod in enumerate(PRODUCTS) if prod[3] == 1 and any(prod[2][0]))

PASS_ORDER = ((11, 6, 14, 0, 7, 9, 4, 12, 2), (1, 8, 3, 13, 9, 5, 6, 12, 10))
STEP_ORDER = (
    'k0 k1 k2 k3 ks v0 v1 r v2 s v3 vs u0 u1 o0 o1 px o2 b2 os u2 u3'.split(),
    'k0 k1 k2 k3 ks v0 v1 r v2 s v3 vs u0 u1 os o0 o1 px o2 b2 u2 u3'.split(),
)
OUT_ORDER = (1, 3, 4, 0, 6, 2, 5)
MIX_PIECES = 4
NEXT_X_AT = 6
OUT_UNROLL = 3


def _dot(a, b):
    return jnp.dot(a, b, preferred_element_type=F32)


def _dot_nt(a, b):
    return lax.dot_general(a, b, (((1,), (1,)), ((), ())), preferred_element_type=F32)


def _dot_split(a, b, parts):
    n = a.shape[0] // parts
    return jnp.concatenate([_dot(a[i * n:(i + 1) * n], b) for i in range(parts)], axis=0)


def _pack(x):
    return pltpu.bitcast(x.astype(BF16), U32)


def _unpack(w):
    return pltpu.bitcast(w, BF16)


def _split_words(words):
    low = lax.bitcast_convert_type(words << 16, F32)
    high = lax.bitcast_convert_type(words & jnp.uint32(0xFFFF0000), F32)
    return low, high


def _tree(op, terms):
    while len(terms) > 1:
        terms = [op(terms[i], terms[i + 1]) if i + 1 < len(terms) else terms[i]
                 for i in range(0, len(terms), 2)]
    return terms[0]


def _combine(terms):
    sign, total = 0, None
    for c, v in terms:
        if not c:
            continue
        if total is None:
            sign, total = c, v
        elif c == sign:
            total = total + v
        elif sign > 0:
            total = total - v
        else:
            sign, total = c, v - total
    return total if sign > 0 else -total


def _layernorm(x, n):
    full = n // LANES * LANES
    lane = lax.broadcasted_iota(jnp.int32, (x.shape[0], LANES), 1)

    def mean(v):
        tiles = [v[:, c:c + LANES] for c in range(0, full, LANES)]
        tiles.append(jnp.where(lane < n - full, v[:, full:], 0.0))
        return jnp.sum(_tree(jnp.add, tiles), axis=1, keepdims=True) * (1.0 / n)

    xc = x - mean(x)
    return xc * lax.rsqrt(mean(xc * xc) + EPS)


def _gelu_twice(u):
    c = 0.7978845608028654
    return u * jnp.tanh(u * (c + (c * 0.044715) * (u * u))) + u


def _group_allreduce(x, op, lane):
    pos = lane & (SUB - 1)
    return _tree(op, [x] + [jnp.where(pos >= j, pltpu.roll(x, j, 1), pltpu.roll(x, LANES - SUB + j, 1))
                            for j in range(1, SUB)])


def _barrel(vs, lane, blk):
    n = len(vs)
    sh = 1
    while sh < n:
        high = (lane & (blk * sh)) != 0
        nxt = []
        for r in range(n):
            a, b = vs[r], vs[(r + sh) % n]
            nxt.append(b if a is None else a if b is None else jnp.where(high, b, a))
        vs = nxt
        sh *= 2
    return vs


def _strassen_lhs(a11, a12, a21, a22):
    return [a11 + a22, a21 + a22, a11, a22, a11 + a12, a21 - a11, a12 - a22]


def _strassen_rhs(b11, b12, b21, b22):
    f11, f12, f21, f22 = (b.astype(F32) for b in (b11, b12, b21, b22))
    return [v.astype(BF16) for v in (f11 + f22, f11, f12 - f22, f21 - f11, f22, f11 + f12, f21 + f22)]


def _strassen_sum(m1, m2, m3, m4, m5, m6, m7):
    return (m1 + m7) + (m4 - m5), m3 + m5, m2 + m4, (m1 + m6) + (m3 - m2)


def _kernel(xT_hbm, mem0_hbm, wq_hbm, wk_hbm, wv_hbm, woT_hbm, w1_hbm, b1_hbm, w2_hbm, b2_hbm,
            outT_hbm,
            wq_s, wk_s, wv_s, wo_s, xT_s, w1_s, w2_s, mem0_s, b1_raw, b2_raw,
            w_main, w_rest, w_qrest, w_krest, w_vrest, w_orest, early_s, early_rest_s, xn_s,
            x_s, h_s, hn_s, hnT_s, lhs_s, u_s, g_s, b2_s, out_s,
            sems, *, seg, scale):
    NP, D, TP = xT_s.shape
    S = NP * TP
    HP = w_orest.shape[0]
    M = mem0_s.shape[0]
    L = M + seg
    F = u_s.shape[1]
    DF = D // LANES * LANES
    DR = D - DF
    NT = DF // LANES
    KG = L // SUB
    SPP = TP // seg
    DH, FH = D // 2, F // 2
    d0, d1 = slice(0, LANES), slice(LANES, 2 * LANES)

    def offset(i, n):
        return i * n if isinstance(i, int) else pl.multiple_of(i * n, n)

    def pair_copy(src, dst, hp):
        return pltpu.make_async_copy(src.bitcast(U32).at[:, hp, :], dst.at[hp], sems.at[hp])

    def qk_copies(hp):
        return [pair_copy(wk_hbm, wk_s, hp), pair_copy(wq_hbm, wq_s, hp)]

    def vo_copies(hp):
        two = pl.ds(2 * hp, 2)
        return [pair_copy(wv_hbm, wv_s, hp),
                pltpu.make_async_copy(woT_hbm.at[two], wo_s.at[two], sems.at[hp])]

    def x_copy(p, sem):
        return pltpu.make_async_copy(xT_hbm.at[:, pl.ds(offset(p, TP), TP)], xT_s.at[p], sem)

    def w1_copy(p):
        return pltpu.make_async_copy(w1_hbm.at[pl.ds(offset(p, TP), TP)], w1_s.at[p], sems.at[p])

    def out_copy(block):
        cols = pl.ds(offset(block, LANES), LANES)
        return pltpu.make_async_copy(out_s.at[:, cols], outT_hbm.at[:, cols], sems.at[HP])

    w2_copy = pltpu.make_async_copy(w2_hbm, w2_s, sems.at[HP])
    small_copies = [pltpu.make_async_copy(src, dst, sems.at[HP]) for src, dst in (
        (mem0_hbm, mem0_s), (b1_hbm, b1_raw), (b2_hbm, b2_raw))] + [x_copy(0, sems.at[HP])]
    for cp in small_copies:
        cp.start()

    def start_qk(hp, c):
        for cp in qk_copies(hp):
            cp.start()
        return c

    lax.fori_loop(0, HP, start_qk, 0)

    def fuse_pair(l0, l1, r0, r1):
        cols = jnp.concatenate([_dot_nt(r0[DF:], l0), _dot_nt(r1[DF:], l1)], axis=0)
        cols = jnp.concatenate([cols, jnp.zeros((LANES, LANES - DR), F32)], axis=1).T[:D]
        a0, a1 = (_dot_nt(jnp.concatenate([l[DF:], l[:DF]], axis=0), r[:DF]) for l, r in ((l0, r0), (l1, r1)))
        return a0[DR:], a1[DR:], cols, jnp.concatenate([a0[:DR], a1[:DR]], axis=0)

    def store_main(unit, a):
        for r, prod in enumerate(PRODUCTS):
            w_main[r, unit] = _pack(_combine(
                [(prod[0][k][n], a[k * LANES:(k + 1) * LANES, n * LANES:(n + 1) * LANES])
                 for k in range(NT) for n in range(NT)]))

    def qk_body(hp, c):
        for cp in qk_copies(hp):
            cp.wait()
        for cp in vo_copies(hp):
            cp.start()
        q0, q1 = _split_words(wq_s[hp])
        k0, k1 = _split_words(wk_s[hp])
        a0, a1, cols, rows = fuse_pair(k0 * scale, k1 * scale, q0, q1)
        store_main(2 * hp, a0)
        store_main(2 * hp + 1, a1)
        rows = rows.T
        for i, w in enumerate(_strassen_rhs(rows[d0], cols[d0], rows[d1], cols[d1])):
            w_rest[i, hp] = pltpu.bitcast(w, U32)
        w_qrest[hp] = _pack(rows[2 * LANES:])
        w_krest[hp] = _pack(cols[2 * LANES:])
        return c

    def vo_body(hp, c):
        for cp in vo_copies(hp):
            cp.wait()
        w1_copy(hp).start()

        @pl.when(hp + 1 < NP)
        def _():
            x_copy(hp + 1, sems.at[hp]).start()

        v0, v1 = _split_words(wv_s[hp])
        a0, a1, cols, rows = fuse_pair(v0, v1, wo_s[2 * hp], wo_s[2 * hp + 1])
        store_main(2 * (HP + hp), a0)
        store_main(2 * (HP + hp) + 1, a1)
        w_vrest[hp] = _pack(cols)
        w_orest[hp] = _pack(rows)
        return c

    def x_rows(p):
        for c in range(0, TP, LANES):
            xT = xT_s[p, :, c:c + LANES].astype(F32)
            x_s[p, c:c + LANES, :] = jnp.concatenate([xT, xT[DF:]], axis=0).T

    def x_pair(p, j):
        return [_layernorm(x_s[p, (j + k) * seg:(j + k + 1) * seg, :], D) for k in range(2)]

    hn_s[0] = jnp.zeros(hn_s.shape[1:], F32)
    h_s[0, TP - seg:, :] = jnp.zeros((seg, h_s.shape[2]), F32)
    for cp in small_copies:
        cp.wait()
    x_rows(0)
    xn_s[0], xn_s[1] = x_pair(0, 0)
    u_s[...] = jnp.broadcast_to(b1_raw[...].astype(F32).reshape(1, F), u_s.shape)
    b2_s[...] = b2_raw[...].astype(F32).reshape(1, S)
    lax.fori_loop(0, HP, qk_body, 0)
    lax.fori_loop(0, HP, vo_body, 0)
    w2_copy.start()

    def all_pairs(ref):
        return _unpack(jnp.concatenate([ref[p] for p in range(HP)], axis=1))

    def main_weights(r, pair):
        return _unpack(jnp.concatenate([w_main[r, 2 * pair], w_main[r, 2 * pair + 1]], axis=1))

    def token_operand(r, xa, xb):
        return _combine([(PRODUCTS[r][1][i][k], x[:, k * LANES:(k + 1) * LANES])
                         for i, x in enumerate((xa, xb)) for k in range(NT)])

    def main_projection(step, mem, now, ahead, saved):
        lhs = {}
        for r, prod in enumerate(PRODUCTS):
            rows = []
            if prod[4 + step] is not None:
                rows.append(_combine([(c, mem[:, k * LANES:(k + 1) * LANES])
                                      for k, c in enumerate(prod[4 + step][0])]))
            if prod[3] == step:
                rows.append(token_operand(r, *(ahead if r in EARLY else now)))
            if rows:
                lhs[r] = jnp.concatenate(rows, axis=0)

        def project(pair):
            prods = {r: _dot(lhs[r], main_weights(r, pair)) for r in PASS_ORDER[step]}
            mem_rows = [_combine([(PRODUCTS[r][4 + step][1][n], v[:M]) for r, v in prods.items()
                                  if PRODUCTS[r][4 + step] is not None]) for n in range(NT)]
            tok = {r: v[-seg:] for r, v in prods.items() if PRODUCTS[r][3] == step}
            if step == 0:
                tok = {**dict(zip(EARLY, saved[pair])), **tok}
                out, saved[pair] = ([_combine([(PRODUCTS[r][2][i][n], v) for r, v in tok.items()])
                                     for n in range(NT)] for i in range(2))
            else:
                out = [_combine([(1, saved[pair][n])] + [(PRODUCTS[r][2][1][n], v) for r, v in tok.items()
                                                         if r not in EARLY]) for n in range(NT)]
                saved[pair] = [tok[r] for r in EARLY]
            full = [jnp.concatenate([m, x], axis=0) for m, x in zip(mem_rows, out)]
            return [[f[:, h * LANES:(h + 1) * LANES] for f in full] for h in range(2)]
        return project

    half = seg // 2

    def rest_dot(m, x, i):
        return _dot(jnp.concatenate([m, x], axis=0), all_pairs(w_rest.at[i]))

    def rest_ahead(xa, xb):
        return xa[:, d1] - xb[:, d1], (xa[:, d0] + xa[:, d1])[half:]

    def rest_projection(step, mem, now, ahead, saved):
        m1, m2 = mem[:, d0], mem[:, d1]
        xa, xb = now

        def project():
            if step == 0:
                p7, p5_rest = saved['rest']
                p1 = rest_dot(m1 + m2, xa[:, d0] + xb[:, d1], 0)
                p3 = rest_dot(m1, xa[:, d0], 2)
                p5 = jnp.concatenate([rest_dot(m1 + m2, (xa[:, d0] + xa[:, d1])[:half], 4), p5_rest], axis=0)
                p4 = rest_dot(m2, xb[:, d1], 3)
                saved['rest'] = (p4[M:], p1[M:] + p3[M:])
                n1 = (p1 + p4) - p5
                return jnp.concatenate([n1[:M], n1[M:] + p7], axis=0), p3 + p5
            t1, t2 = saved['rest']
            x7, x5 = rest_ahead(*ahead)
            p2 = rest_dot(m1, xb[:, d0] + xb[:, d1], 1)
            p6 = rest_dot(m1, xb[:, d0] - xa[:, d0], 5)
            p5 = rest_dot(m2, x5, 4)
            p7 = rest_dot(m2, x7, 6)
            saved['rest'] = (p7[M:], p5[M:])
            return (p2 + jnp.concatenate([p7[:M] - p5[:M], t1], axis=0),
                    (p6 - p2) + jnp.concatenate([p5[:M], t2], axis=0))
        return project

    def segment(order, xs, mem, project, project_rest, filler, neg):
        row = lax.broadcasted_iota(jnp.int32, (L, LANES), 0)
        lane = lax.broadcasted_iota(jnp.int32, (L, LANES), 1)
        low = lane < DR
        blk = 2 * SUB
        hs = jnp.concatenate([mem, xs], axis=0)
        res = {}

        def stack(heads):
            return jnp.concatenate([h[g * SUB:(g + 1) * SUB] for g in range(KG) for h in heads], axis=0)

        def main_tile(kind, t):
            return [head[t] for i in range(HP // 2) for head in res[kind + str(i)]]

        def by_head(shared):
            out = []
            for p in range(HP):
                t = shared[:, p * LANES:(p + 1) * LANES]
                out += [jnp.where(low, t, 0.0), jnp.where(low, 0.0, t)]
            return out

        first, second = jnp.where(low, hs[:, DF:], 0.0), jnp.where(low, 0.0, hs[:, DF:])
        keys = [jnp.concatenate([first[g * SUB:(g + 1) * SUB], second[g * SUB:(g + 1) * SUB]], axis=0)
                for g in range(KG)] + [jnp.zeros((blk, LANES), F32)] * (HP - KG)

        def scores_rest():
            q = jnp.concatenate([res['q'][:, p * LANES:(p + 1) * LANES] for p in range(HP)], axis=0)
            r = _dot(q, jnp.concatenate(keys, axis=0).T.astype(BF16))
            r = [r[p * L:(p + 1) * L] for p in range(HP)]
            r = _barrel([pltpu.roll(t, blk * p, 1) if p else t for p, t in enumerate(r)], lane, blk)
            return [pltpu.roll(r[-g % HP], LANES - blk * g, 1) if g else r[0] for g in range(KG)]

        def scores_main():
            k = jnp.concatenate([stack(main_tile('k', t)) for t in range(NT)] + [stack(by_head(res['ks']))],
                                axis=1)
            out = []
            for g in range(KG):
                begin = max(M, g * SUB)
                t = _dot(jnp.concatenate([hs[:M], hs[begin:]], axis=0),
                         k[g * LANES:(g + 1) * LANES].T.astype(BF16))
                gap = [jnp.zeros((begin - M, LANES), F32)] if begin > M else []
                out.append(jnp.concatenate([t[:M]] + gap + [t[M:]], axis=0))
            return out

        def softmax():
            if 'p' not in res:
                tiles = []
                for g in range(KG):
                    key = g * SUB + (lane & (SUB - 1))
                    tiles.append(jnp.where((row < M) | (row >= key), res['s'][g] + res['r'][g], neg))
                top = _group_allreduce(functools.reduce(jnp.maximum, tiles), jnp.maximum, lane)
                ex = [jnp.exp(t - top) for t in tiles]
                inv = 1.0 / _group_allreduce(functools.reduce(jnp.add, ex), jnp.add, lane)
                res['p'] = [e * inv for e in ex]
            return res['p']

        def mix_rest():
            p = [pltpu.roll(t, blk * g, 1) if g else t for g, t in enumerate(softmax())]
            p = _barrel(p + [None] * (HP - KG), lane, blk)
            return jnp.concatenate(
                [_dot(p[-i % HP], jnp.concatenate([keys[(j - i) % HP] for j in range(HP)], axis=0).astype(BF16))
                 for i in range(HP)], axis=1)

        def mix(values):
            return _dot(jnp.concatenate(softmax(), axis=1), stack(values).astype(BF16))

        for name in order:
            if name == 'ks':
                q, k = project_rest()
                res['ks'] = k + _dot(hs[:, 2 * LANES:D], all_pairs(w_krest))
                res['q'] = q + _dot(hs[:, 2 * LANES:DF], all_pairs(w_qrest))
            elif name == 'vs':
                res[name] = _dot(hs[:, :D], all_pairs(w_vrest))
            elif name[0] in 'kv':
                pair = HP * (name[0] == 'v') + 2 * int(name[1])
                res[name] = project(pair) + project(pair + 1)
            elif name == 'r':
                res[name] = scores_rest()
            elif name == 's':
                res[name] = scores_main()
            elif name == 'px':
                res[name] = mix_rest()
            elif name == 'b2':
                res[name] = _dot(res['px'], _unpack(jnp.concatenate([w_orest[p] for p in range(HP)], axis=0)))
            elif name == 'os':
                res[name] = mix(by_head(res['vs']))
            elif name[0] == 'o':
                res[name] = mix(main_tile('v', int(name[1])))
            else:
                filler(int(name[1]))
        o = jnp.concatenate([res['o%d' % t] for t in range(NT)], axis=1) + res['b2']
        o = jnp.concatenate([o, res['os'] + pltpu.roll(res['os'], DR, 1)], axis=1)
        return o[:M], o[M:]

    def mixer_norm(h):
        return _layernorm(_layernorm(h, D), D)

    def transpose_hn(slot, c):
        hnT_s[:, c:c + LANES] = hn_s[slot, c:c + LANES, :].T[:D]

    def mixer_operands():
        ops = _strassen_lhs(hnT_s[:DH, d0], hnT_s[:DH, d1], hnT_s[DH:, d0], hnT_s[DH:, d1])
        for i, a in enumerate(ops):
            lhs_s[i] = a

    def hidden_cols(t):
        return slice(t * LANES, (t + 1) * LANES), slice(FH + t * LANES, FH + (t + 1) * LANES)

    def w1_operands(p, c1, c2):
        return _strassen_rhs(w1_s[p, d0, c1], w1_s[p, d0, c2], w1_s[p, d1, c1], w1_s[p, d1, c2])

    def accumulate(p, t, piece):
        c1, c2 = hidden_cols(t)
        rhs = w1_operands(p, c1, c2)
        n = DH // MIX_PIECES
        top, bot = slice(piece * n, (piece + 1) * n), slice(DH + piece * n, DH + (piece + 1) * n)
        c11, c12, c21, c22 = _strassen_sum(*[_dot(lhs_s[i, top], rhs[i]) for i in range(7)])
        u_s[top, c1] += c11
        u_s[top, c2] += c12
        u_s[bot, c1] += c21
        u_s[bot, c2] += c22

    def pair_cols(pair):
        return slice(2 * pair * LANES, 2 * (pair + 1) * LANES)

    def pair_body(p, mem):
        w1_copy(p).wait()

        @pl.when(p + 1 < NP)
        def _():
            x_copy(p + 1, sems.at[p]).wait()

        prev, following = jnp.maximum(p - 1, 0), jnp.minimum(p + 1, NP - 1)
        zero = jnp.minimum(p, 0)

        def mask_value_after(ref):
            return jnp.concatenate([jnp.where(p < 0, ref[zero, :SUB, :LANES], NEG)] * KG, axis=0)

        saved = {pair: [early_s[i, :, pair_cols(pair)] for i in range(len(EARLY))] for pair in range(2 * HP)}
        saved['rest'] = (early_rest_s[:seg], early_rest_s[seg:])
        now = xn_s[0], xn_s[1]
        for j in range(SPP):
            rows = slice(j * seg, (j + 1) * seg)
            x = x_s[p, rows, :]
            if j == 0:
                hn_s[p, TP - seg:, :] = mixer_norm(h_s[p, TP - seg:, :])
                for c in range(0, TP, LANES):
                    transpose_hn(p, c)
                mixer_operands()
            else:
                hn_s[p + 1, (j - 1) * seg:j * seg, :] = mixer_norm(h)
            if j == NEXT_X_AT:
                x_rows(following)
            step, tile = j % 2, j - (SPP - FH // LANES)
            ahead = None
            if step:
                ahead = x_pair(p, j + 1) if j + 1 < SPP else x_pair(following, 0)
            args = (step, mem, now, ahead, saved)
            mem, att = segment(STEP_ORDER[step], now[step], mem, main_projection(*args), rest_projection(*args),
                               functools.partial(accumulate, prev, tile) if tile >= 0 else lambda piece: None,
                               mask_value_after(hn_s))
            if step:
                now = ahead
            h = x + att
            h_s[p + 1, rows, :] = h
        xn_s[0], xn_s[1] = now
        early_rest_s[:seg], early_rest_s[seg:] = saved['rest']
        for pair in range(2 * HP):
            for i, v in enumerate(saved[pair]):
                early_s[i, :, pair_cols(pair)] = v
        return mem

    start = xn_s[0], xn_s[1]
    x7, x5 = rest_ahead(*start)
    early_rest_s[:seg], early_rest_s[seg:] = _dot(x7, all_pairs(w_rest.at[6])), _dot(x5, all_pairs(w_rest.at[4]))
    for i, r in enumerate(EARLY):
        for pair in range(2 * HP):
            early_s[i, :, pair_cols(pair)] = _dot(token_operand(r, *start), main_weights(r, pair))
    mem0 = mem0_s[...].astype(F32)
    lax.fori_loop(0, NP, pair_body, jnp.concatenate([mem0, mem0[:, DF:]], axis=1))

    def out_cols(p):
        return pl.ds(offset(2 * p, LANES), LANES), pl.ds(offset(2 * p + 1, LANES), LANES)

    def w2_operands(p, k1, k2):
        n1, n2 = out_cols(p)
        return _strassen_rhs(w2_s[k1, n1], w2_s[k1, n2], w2_s[k2, n1], w2_s[k2, n2])

    def out_store(p, c11, c12, c21, c22):
        for k, (cols, top, bot) in enumerate(zip(out_cols(p), (c11, c12), (c21, c22))):
            h = h_s[p + 1, k * LANES:(k + 1) * LANES, :].T[:D]
            y = jnp.concatenate([top, bot], axis=0)
            out_s[:, cols] = (h + (0.5 * y + b2_s[:, cols])).astype(out_s.dtype)
            out_copy(2 * p + k).start()

    def out_block(p):
        rhs = w2_operands(p, slice(0, FH), slice(FH, F))
        m = {i: _dot(g_s[i], rhs[i]) for i in OUT_ORDER}
        out_store(p, *_strassen_sum(*[m[i] for i in range(7)]))

    w2_copy.wait()
    tiles = [hidden_cols(t) for t in range(FH // LANES)]
    transpose_hn(NP, 0)
    x11, x21 = hnT_s[:DH, d0], hnT_s[DH:, d0]
    for c1, c2 in tiles:
        rhs = w1_operands(NP - 1, c1, c2)
        m3, m6 = _dot_split(x11, rhs[2], 2), _dot_split(x21 - x11, rhs[5], 2)
        u_s[:DH, c2] += m3
        u_s[DH:, c2] += m3 + m6
    hn_s[NP, TP - seg:, :] = mixer_norm(h_s[NP, TP - seg:, :])
    transpose_hn(NP, LANES)
    mixer_operands()

    acc, ready = None, []

    def drain(acc):
        k1 = slice(ready[0][1].start, ready[-1][1].stop)
        k2 = slice(ready[0][2].start, ready[-1][2].stop)
        lhs = [jnp.concatenate([r[0][i] for r in ready], axis=1) for i in range(7)]
        prods = [_dot_split(a, b, 2) for a, b in zip(lhs, w2_operands(0, k1, k2))]
        ready.clear()
        return prods if acc is None else [a + b for a, b in zip(acc, prods)]

    for t, (c1, c2) in enumerate(tiles):
        rhs = w1_operands(NP - 1, c1, c2)
        m1, m2, m4, m5, m7 = (_dot_split(lhs_s[i], rhs[i], MIX_PIECES) for i in (0, 1, 3, 4, 6))
        if t and t % 2 == 0:
            acc = drain(acc)
        ops = _strassen_lhs(_gelu_twice(u_s[:DH, c1] + ((m1 + m7) + (m4 - m5))), _gelu_twice(u_s[:DH, c2] + m5),
                            _gelu_twice(u_s[DH:, c1] + (m2 + m4)), _gelu_twice(u_s[DH:, c2] + (m1 - m2)))
        for i, a in enumerate(ops):
            g_s[i, :, c1] = a
        ready.append((ops, c1, c2))
    out_store(0, *_strassen_sum(*drain(acc)))
    peeled = 1 + (NP - 1) % OUT_UNROLL
    for p in range(1, peeled):
        out_block(p)

    def out_body(i, c):
        for k in range(OUT_UNROLL):
            out_block(peeled + i * OUT_UNROLL + k)
        return c

    if NP > peeled:
        lax.fori_loop(0, (NP - peeled) // OUT_UNROLL, out_body, 0)
    for block in range(2 * NP):
        out_copy(block).wait()


@functools.partial(jax.jit, static_argnames=("A_seg_len",))
def pallas_sequential_preLN__memory_aug_recurrent_mem_tr__mixer_token_mlp__prompt_kernel(
        A_x, A_mem0, A_Wq, A_Wk, A_Wv, A_Wo, A_seg_len, B_x, B_w1, B_b1, B_w2, B_b2):
    del B_x
    B, S, D = A_x.shape
    _, H, E = A_Wq.shape
    M = A_mem0.shape[1]
    F = B_w1.shape[1]
    seg = int(A_seg_len)
    HP = H // 2
    DF = D // LANES * LANES
    DP = DF + LANES
    TP = 2 * LANES
    NP = S // TP
    assert B == 1 and M == SUB and seg == 4 * SUB and H * SUB == LANES
    assert DF == 3 * LANES and 2 * (D - DF) == LANES and S == HP * TP and F == 7 * TP
    hbm = pl.BlockSpec(memory_space=pl.ANY)
    outT = pl.pallas_call(
        functools.partial(_kernel, seg=seg, scale=E ** -0.5),
        out_shape=jax.ShapeDtypeStruct((D, S), A_x.dtype),
        in_specs=[hbm] * 10,
        out_specs=hbm,
        scratch_shapes=[
            pltpu.VMEM((HP, D, E), U32),
            pltpu.VMEM((HP, D, E), U32),
            pltpu.VMEM((HP, D, E), U32),
            pltpu.VMEM((H, D, E), BF16),
            pltpu.VMEM((NP, D, TP), BF16),
            pltpu.VMEM((NP, TP, F), BF16),
            pltpu.VMEM((F, S), BF16),
            pltpu.VMEM((M, D), BF16),
            pltpu.VMEM((F,), BF16),
            pltpu.VMEM((S,), BF16),
            pltpu.VMEM((len(PRODUCTS), 2 * H, LANES // 2, LANES), U32),
            pltpu.VMEM((7, HP, LANES // 2, LANES), U32),
            pltpu.VMEM((HP, LANES // 2, LANES), U32),
            pltpu.VMEM((HP, (D - 2 * LANES) // 2, LANES), U32),
            pltpu.VMEM((HP, D // 2, LANES), U32),
            pltpu.VMEM((HP, LANES // 2, DF), U32),
            pltpu.VMEM((len(EARLY), seg, 2 * H * LANES), F32),
            pltpu.VMEM((seg + seg // 2, HP * LANES), F32),
            pltpu.VMEM((2, seg, DP), F32),
            pltpu.VMEM((NP, TP, DP), F32),
            pltpu.VMEM((NP + 1, TP, DP), F32),
            pltpu.VMEM((NP + 1, TP, DP), F32),
            pltpu.VMEM((D, TP), F32),
            pltpu.VMEM((7, D // 2, LANES), F32),
            pltpu.VMEM((D, F), F32),
            pltpu.VMEM((7, D // 2, F // 2), F32),
            pltpu.VMEM((1, S), F32),
            pltpu.VMEM((D, S), A_x.dtype),
            pltpu.SemaphoreType.DMA((HP + 1,)),
        ],
        compiler_params=pltpu.CompilerParams(vmem_limit_bytes=110 * 2**20),
    )(
        jnp.swapaxes(A_x, 1, 2).reshape(D, S),
        A_mem0.reshape(M, D),
        A_Wq, A_Wk, A_Wv,
        jnp.swapaxes(A_Wo, 1, 2),
        B_w1, B_b1, B_w2, B_b2,
    )
    return jnp.swapaxes(outT.reshape(B, D, S), 1, 2)
```

```python
import functools

import jax
import jax.numpy as jnp
import numpy as np
from jax import lax
import jax.experimental.pallas as pl
import jax.experimental.pallas.tpu as pltpu

LANES = 128
SUB = 8
EPS = 1e-5
NEG = -1000000000.0
F32 = jnp.float32
BF16 = jnp.bfloat16
U32 = jnp.uint32

PRODUCTS = (
    (((1, -1, 0), (0, 0, 0), (-1, 0, 0)), ((1, 0, 0), (0, 0, 0)), ((1, 0, 0), (-1, 0, 0)),
     0, ((1, 0, 0), (1, 0, 0)), None),
    (((1, 0, -1), (-1, 0, 0), (0, 0, 0)), ((1, 0, 0), (1, 0, 0)), ((0, 0, 0), (1, 0, 0)),
     1, None, ((1, 0, 0), (1, 0, 0))),
    (((0, 0, 0), (-1, 1, 0), (0, -1, 0)), ((0, 1, 0), (0, 0, 0)), ((0, 1, 0), (0, 0, 0)),
     0, ((0, 1, 0), (0, 1, 0)), None),
    (((0, -1, 0), (0, 1, 1), (0, 0, 0)), ((0, 0, 0), (0, 1, 0)), ((0, 0, 0), (0, 1, 0)),
     1, None, ((0, 1, 0), (0, 1, 0))),
    (((0, 0, 0), (0, 0, -1), (-1, 0, 1)), ((0, 0, 1), (0, 0, 1)), ((0, 0, 1), (0, 0, 0)),
     0, ((0, 0, 1), (0, 0, 1)), None),
    (((0, 0, 1), (0, 0, 0), (0, -1, -1)), ((0, 0, 0), (0, 0, 1)), ((0, 0, 1), (0, 0, -1)),
     1, None, ((0, 0, 1), (0, 0, -1))),
    (((0, 0, 0), (1, 0, 0), (0, 0, 0)), ((1, 1, 0), (1, 1, 0)), ((1, 1, 0), (0, 0, 0)),
     0, ((1, 1, 0), (1, 1, 0)), ((1, 1, 0), (1, 0, 0))),
    (((0, 1, 0), (-1, 0, 0), (0, 0, 0)), ((1, 0, 0), (1, 1, 0)), ((1, 1, 0), (-1, 0, 0)),
     0, ((1, 0, 0), (1, 1, 0)), None),
    (((0, 1, 0), (0, 0, 0), (0, 0, 0)), ((0, 0, 0), (1, 1, 0)), ((-1, -1, 0), (1, 1, 0)),
     1, None, ((1, 1, 0), (0, 1, 0))),
    (((0, 0, 0), (0, 0, 1), (0, 0, 0)), ((0, 1, 1), (0, 1, 1)), ((0, 0, 0), (0, -1, 1)),
     1, ((0, 1, 1), (0, 0, 1)), ((0, 1, 1), (0, -1, 1))),
    (((0, 0, 0), (0, 0, 1), (0, 1, 0)), ((0, 1, 1), (0, 0, 1)), ((0, 0, 1), (0, 1, -1)),
     1, None, ((0, 0, 1), (0, 1, -1))),
    (((0, 0, 0), (0, 0, 0), (0, 1, 0)), ((0, 1, 1), (0, 0, 0)), ((0, 1, -1), (0, -1, 1)),
     0, ((0, 1, 1), (0, 1, 0)), None),
    (((0, 0, 1), (0, 0, 0), (-1, 0, 0)), ((1, 0, 0), (0, 0, -1)), ((0, 0, 1), (1, 0, 0)),
     0, ((1, 0, 0), (0, 0, 1)), ((0, 0, 1), (-1, 0, 0))),
    (((0, 0, 1), (0, 0, 0), (0, 0, 0)), ((0, 0, 0), (1, 0, 1)), ((0, 0, 0), (1, 0, 1)),
     1, None, ((1, 0, 1), (1, 0, 1))),
    (((0, 0, 0), (0, 0, 0), (1, 0, 0)), ((1, 0, 1), (0, 0, 0)), ((1, 0, 1), (0, 0, 0)),
     0, ((1, 0, 1), (1, 0, 1)), None),
)
EARLY = tuple(r for r, prod in enumerate(PRODUCTS) if prod[3] == 1 and any(prod[2][0]))

PASS_ORDER = ((11, 6, 14, 0, 7, 9, 4, 12, 2), (1, 8, 3, 13, 9, 5, 6, 12, 10))
STEP_ORDER = (
    'v0 k0 k1 k2 k3 ks v1 r v2 s v3 vs u0 u1 o0 o1 px o2 b2 os u2 u3'.split(),
    'k0 k1 k2 k3 ks v0 v1 r v2 s v3 vs u0 u1 o0 os o1 px o2 b2 u2 u3'.split(),
)
OUT_ORDER = (1, 3, 4, 0, 6, 2, 5)
MIX_PIECES = 4
NEXT_X_AT = 6
OUT_UNROLL = 3


def _dot(a, b):
    return jnp.dot(a, b, preferred_element_type=F32)


def _dot_nt(a, b):
    return lax.dot_general(a, b, (((1,), (1,)), ((), ())), preferred_element_type=F32)


def _dot_split(a, b, parts):
    n = a.shape[0] // parts
    return jnp.concatenate([_dot(a[i * n:(i + 1) * n], b) for i in range(parts)], axis=0)


def _pack(x):
    return pltpu.bitcast(x.astype(BF16), U32)


def _unpack(w):
    return pltpu.bitcast(w, BF16)


def _split_words(words):
    low = lax.bitcast_convert_type(words << 16, F32)
    high = lax.bitcast_convert_type(words & np.uint32(0xFFFF0000), F32)
    return low, high


def _tree(op, terms):
    while len(terms) > 1:
        terms = [op(terms[i], terms[i + 1]) if i + 1 < len(terms) else terms[i]
                 for i in range(0, len(terms), 2)]
    return terms[0]


def _combine(terms):
    sign, total = 0, None
    for c, v in terms:
        if not c:
            continue
        if total is None:
            sign, total = c, v
        elif c == sign:
            total = total + v
        elif sign > 0:
            total = total - v
        else:
            sign, total = c, v - total
    return total if sign > 0 else -total


def _layernorm(x, n):
    full = n // LANES * LANES
    lane = lax.broadcasted_iota(jnp.int32, (x.shape[0], LANES), 1)

    def mean(v):
        tiles = [v[:, c:c + LANES] for c in range(0, full, LANES)]
        tiles.append(jnp.where(lane < n - full, v[:, full:], 0.0))
        return jnp.sum(_tree(jnp.add, tiles), axis=1, keepdims=True) * (1.0 / n)

    xc = x - mean(x)
    return xc * lax.rsqrt(mean(xc * xc) + EPS)


def _gelu_twice(u):
    c = 0.7978845608028654
    return u * jnp.tanh(u * (c + (c * 0.044715) * (u * u))) + u


def _group_allreduce(x, op, lane):
    pos = lane & (SUB - 1)
    return _tree(op, [x] + [jnp.where(pos >= j, pltpu.roll(x, j, 1), pltpu.roll(x, LANES - SUB + j, 1))
                            for j in range(1, SUB)])


def _barrel(vs, lane, blk):
    n = len(vs)
    sh = 1
    while sh < n:
        high = (lane & (blk * sh)) != 0
        nxt = []
        for r in range(n):
            a, b = vs[r], vs[(r + sh) % n]
            nxt.append(b if a is None else a if b is None else jnp.where(high, b, a))
        vs = nxt
        sh *= 2
    return vs


def _strassen_lhs(a11, a12, a21, a22):
    return [a11 + a22, a21 + a22, a11, a22, a11 + a12, a21 - a11, a12 - a22]


def _strassen_rhs(b11, b12, b21, b22):
    f11, f12, f21, f22 = (b.astype(F32) for b in (b11, b12, b21, b22))
    return [v.astype(BF16) for v in (f11 + f22, f11, f12 - f22, f21 - f11, f22, f11 + f12, f21 + f22)]


def _strassen_sum(m1, m2, m3, m4, m5, m6, m7):
    return (m1 + m7) + (m4 - m5), m3 + m5, m2 + m4, (m1 + m6) + (m3 - m2)


def _kernel(xT_hbm, mem0_hbm, wq_hbm, wk_hbm, wv_hbm, woT_hbm, w1_hbm, b1_hbm, w2_hbm, b2_hbm,
            outT_hbm,
            wq_s, wk_s, wv_s, wo_s, xT_s, w1_s, w2_s, mem0_s, b1_raw, b2_raw,
            w_main, w_rest, w_qrest, w_krest, w_vrest, w_orest, early_s, early_rest_s, xn_s,
            x_s, h_s, hn_s, hnT_s, lhs_s, u_s, g_s, b2_s, out_s,
            sems, *, seg, scale):
    NP, D, TP = xT_s.shape
    S = NP * TP
    HP = w_orest.shape[0]
    M = mem0_s.shape[0]
    L = M + seg
    F = u_s.shape[1]
    DF = D // LANES * LANES
    DR = D - DF
    NT = DF // LANES
    KG = L // SUB
    SPP = TP // seg
    DH, FH = D // 2, F // 2
    d0, d1 = slice(0, LANES), slice(LANES, 2 * LANES)

    def offset(i, n):
        return i * n if isinstance(i, int) else pl.multiple_of(i * n, n)

    def pair_copy(src, dst, hp):
        return pltpu.make_async_copy(src.bitcast(U32).at[:, hp, :], dst.at[hp], sems.at[hp])

    def qk_copies(hp):
        return [pair_copy(wk_hbm, wk_s, hp), pair_copy(wq_hbm, wq_s, hp)]

    def vo_copies(hp):
        two = pl.ds(2 * hp, 2)
        return [pair_copy(wv_hbm, wv_s, hp),
                pltpu.make_async_copy(woT_hbm.at[two], wo_s.at[two], sems.at[hp])]

    def x_copy(p, sem):
        return pltpu.make_async_copy(xT_hbm.at[:, pl.ds(offset(p, TP), TP)], xT_s.at[p], sem)

    def w1_copy(p):
        return pltpu.make_async_copy(w1_hbm.at[pl.ds(offset(p, TP), TP)], w1_s.at[p], sems.at[p])

    def out_copy(block):
        cols = pl.ds(offset(block, LANES), LANES)
        return pltpu.make_async_copy(out_s.at[:, cols], outT_hbm.at[:, cols], sems.at[HP])

    w2_copy = pltpu.make_async_copy(w2_hbm, w2_s, sems.at[HP])
    small_copies = [pltpu.make_async_copy(src, dst, sems.at[HP]) for src, dst in (
        (mem0_hbm, mem0_s), (b1_hbm, b1_raw), (b2_hbm, b2_raw))] + [x_copy(0, sems.at[HP])]
    for cp in small_copies:
        cp.start()

    def start_qk(hp, c):
        for cp in qk_copies(hp):
            cp.start()
        return c

    lax.fori_loop(0, HP, start_qk, 0)

    def fuse_pair(l0, l1, r0, r1):
        cols = jnp.concatenate([_dot_nt(r0[DF:], l0), _dot_nt(r1[DF:], l1)], axis=0)
        cols = jnp.concatenate([cols, jnp.zeros((LANES, LANES - DR), F32)], axis=1).T[:D]
        a0, a1 = (_dot_nt(jnp.concatenate([l[DF:], l[:DF]], axis=0), r[:DF]) for l, r in ((l0, r0), (l1, r1)))
        return a0[DR:], a1[DR:], cols, jnp.concatenate([a0[:DR], a1[:DR]], axis=0)

    def store_main(unit, a):
        for r, prod in enumerate(PRODUCTS):
            w_main[r, unit] = _pack(_combine(
                [(prod[0][k][n], a[k * LANES:(k + 1) * LANES, n * LANES:(n + 1) * LANES])
                 for k in range(NT) for n in range(NT)]))

    def qk_body(hp, c):
        for cp in qk_copies(hp):
            cp.wait()
        for cp in vo_copies(hp):
            cp.start()
        q0, q1 = _split_words(wq_s[hp])
        k0, k1 = _split_words(wk_s[hp])
        a0, a1, cols, rows = fuse_pair(k0 * scale, k1 * scale, q0, q1)
        store_main(2 * hp, a0)
        store_main(2 * hp + 1, a1)
        rows = rows.T
        for i, w in enumerate(_strassen_rhs(rows[d0], cols[d0], rows[d1], cols[d1])):
            w_rest[i, hp] = pltpu.bitcast(w, U32)
        w_qrest[hp] = _pack(rows[2 * LANES:])
        w_krest[hp] = _pack(cols[2 * LANES:])
        return c

    def vo_body(hp, c):
        for cp in vo_copies(hp):
            cp.wait()
        w1_copy(hp).start()

        @pl.when(hp + 1 < NP)
        def _():
            x_copy(hp + 1, sems.at[hp]).start()

        v0, v1 = _split_words(wv_s[hp])
        a0, a1, cols, rows = fuse_pair(v0, v1, wo_s[2 * hp], wo_s[2 * hp + 1])
        store_main(2 * (HP + hp), a0)
        store_main(2 * (HP + hp) + 1, a1)
        w_vrest[hp] = _pack(cols)
        w_orest[hp] = _pack(rows)
        return c

    def x_rows(p):
        for c in range(0, TP, LANES):
            xT = xT_s[p, :, c:c + LANES].astype(F32)
            x_s[p, c:c + LANES, :] = jnp.concatenate([xT, xT[DF:]], axis=0).T

    def x_pair(p, j):
        return [_layernorm(x_s[p, (j + k) * seg:(j + k + 1) * seg, :], D) for k in range(2)]

    hn_s[0] = jnp.zeros(hn_s.shape[1:], F32)
    h_s[0, TP - seg:, :] = jnp.zeros((seg, h_s.shape[2]), F32)
    for cp in small_copies:
        cp.wait()
    x_rows(0)
    xn_s[0], xn_s[1] = x_pair(0, 0)
    u_s[...] = jnp.broadcast_to(b1_raw[...].astype(F32).reshape(1, F), u_s.shape)
    b2_s[...] = b2_raw[...].astype(F32).reshape(1, S)
    lax.fori_loop(0, HP, qk_body, 0)
    lax.fori_loop(0, HP, vo_body, 0)
    w2_copy.start()

    def all_pairs(ref):
        return _unpack(jnp.concatenate([ref[p] for p in range(HP)], axis=1))

    def main_weights(r, pair):
        return _unpack(jnp.concatenate([w_main[r, 2 * pair], w_main[r, 2 * pair + 1]], axis=1))

    def token_operand(r, xa, xb):
        return _combine([(PRODUCTS[r][1][i][k], x[:, k * LANES:(k + 1) * LANES])
                         for i, x in enumerate((xa, xb)) for k in range(NT)])

    def main_projection(step, mem, now, ahead, saved):
        lhs = {}
        for r, prod in enumerate(PRODUCTS):
            rows = []
            if prod[4 + step] is not None:
                rows.append(_combine([(c, mem[:, k * LANES:(k + 1) * LANES])
                                      for k, c in enumerate(prod[4 + step][0])]))
            if prod[3] == step:
                rows.append(token_operand(r, *(ahead if r in EARLY else now)))
            if rows:
                lhs[r] = jnp.concatenate(rows, axis=0)

        def project(pair):
            prods = {r: _dot(lhs[r], main_weights(r, pair)) for r in PASS_ORDER[step]}
            mem_rows = [_combine([(PRODUCTS[r][4 + step][1][n], v[:M]) for r, v in prods.items()
                                  if PRODUCTS[r][4 + step] is not None]) for n in range(NT)]
            tok = {r: v[-seg:] for r, v in prods.items() if PRODUCTS[r][3] == step}
            if step == 0:
                tok = {**dict(zip(EARLY, saved[pair])), **tok}
                out, saved[pair] = ([_combine([(PRODUCTS[r][2][i][n], v) for r, v in tok.items()])
                                     for n in range(NT)] for i in range(2))
            else:
                out = [_combine([(1, saved[pair][n])] + [(PRODUCTS[r][2][1][n], v) for r, v in tok.items()
                                                         if r not in EARLY]) for n in range(NT)]
                saved[pair] = [tok[r] for r in EARLY]
            full = [jnp.concatenate([m, x], axis=0) for m, x in zip(mem_rows, out)]
            return [[f[:, h * LANES:(h + 1) * LANES] for f in full] for h in range(2)]
        return project

    half = seg // 2

    def rest_dot(m, x, i):
        return _dot(jnp.concatenate([m, x], axis=0), all_pairs(w_rest.at[i]))

    def rest_ahead(xa, xb):
        return xa[:, d1] - xb[:, d1], (xa[:, d0] + xa[:, d1])[half:]

    def rest_projection(step, mem, now, ahead, saved):
        m1, m2 = mem[:, d0], mem[:, d1]
        xa, xb = now

        def project():
            if step == 0:
                p7, p5_rest = saved['rest']
                p1 = rest_dot(m1 + m2, xa[:, d0] + xb[:, d1], 0)
                p3 = rest_dot(m1, xa[:, d0], 2)
                p5 = jnp.concatenate([rest_dot(m1 + m2, (xa[:, d0] + xa[:, d1])[:half], 4), p5_rest], axis=0)
                p4 = rest_dot(m2, xb[:, d1], 3)
                saved['rest'] = (p4[M:], p1[M:] + p3[M:])
                n1 = (p1 + p4) - p5
                return jnp.concatenate([n1[:M], n1[M:] + p7], axis=0), p3 + p5
            t1, t2 = saved['rest']
            x7, x5 = rest_ahead(*ahead)
            p2 = rest_dot(m1, xb[:, d0] + xb[:, d1], 1)
            p6 = rest_dot(m1, xb[:, d0] - xa[:, d0], 5)
            p5 = rest_dot(m2, x5, 4)
            p7 = rest_dot(m2, x7, 6)
            saved['rest'] = (p7[M:], p5[M:])
            return (p2 + jnp.concatenate([p7[:M] - p5[:M], t1], axis=0),
                    (p6 - p2) + jnp.concatenate([p5[:M], t2], axis=0))
        return project

    def segment(order, xs, mem, project, project_rest, filler, neg):
        row = lax.broadcasted_iota(jnp.int32, (L, LANES), 0)
        lane = lax.broadcasted_iota(jnp.int32, (L, LANES), 1)
        low = lane < DR
        blk = 2 * SUB
        hs = jnp.concatenate([mem, xs], axis=0)
        res = {}

        def stack(heads):
            return jnp.concatenate([h[g * SUB:(g + 1) * SUB] for g in range(KG) for h in heads], axis=0)

        def main_tile(kind, t):
            return [head[t] for i in range(HP // 2) for head in res[kind + str(i)]]

        def by_head(shared):
            out = []
            for p in range(HP):
                t = shared[:, p * LANES:(p + 1) * LANES]
                out += [jnp.where(low, t, 0.0), jnp.where(low, 0.0, t)]
            return out

        first, second = jnp.where(low, hs[:, DF:], 0.0), jnp.where(low, 0.0, hs[:, DF:])
        keys = [jnp.concatenate([first[g * SUB:(g + 1) * SUB], second[g * SUB:(g + 1) * SUB]], axis=0)
                for g in range(KG)] + [jnp.zeros((blk, LANES), F32)] * (HP - KG)

        def scores_rest():
            q = jnp.concatenate([res['q'][:, p * LANES:(p + 1) * LANES] for p in range(HP)], axis=0)
            r = _dot(q, jnp.concatenate(keys, axis=0).T.astype(BF16))
            r = [r[p * L:(p + 1) * L] for p in range(HP)]
            r = _barrel([pltpu.roll(t, blk * p, 1) if p else t for p, t in enumerate(r)], lane, blk)
            return [pltpu.roll(r[-g % HP], LANES - blk * g, 1) if g else r[0] for g in range(KG)]

        def scores_main():
            k = jnp.concatenate([stack(main_tile('k', t)) for t in range(NT)] + [stack(by_head(res['ks']))],
                                axis=1)
            out = []
            for g in range(KG):
                begin = max(M, g * SUB)
                t = _dot(jnp.concatenate([hs[:M], hs[begin:]], axis=0),
                         k[g * LANES:(g + 1) * LANES].T.astype(BF16))
                gap = [jnp.zeros((begin - M, LANES), F32)] if begin > M else []
                out.append(jnp.concatenate([t[:M]] + gap + [t[M:]], axis=0))
            return out

        def softmax():
            if 'p' not in res:
                tiles = []
                for g in range(KG):
                    key = g * SUB + (lane & (SUB - 1))
                    tiles.append(jnp.where((row < M) | (row >= key), res['s'][g] + res['r'][g], neg))
                top = _group_allreduce(functools.reduce(jnp.maximum, tiles), jnp.maximum, lane)
                ex = [jnp.exp(t - top) for t in tiles]
                inv = 1.0 / _group_allreduce(functools.reduce(jnp.add, ex), jnp.add, lane)
                res['p'] = [e * inv for e in ex]
            return res['p']

        def mix_rest():
            p = [pltpu.roll(t, blk * g, 1) if g else t for g, t in enumerate(softmax())]
            p = _barrel(p + [None] * (HP - KG), lane, blk)
            return jnp.concatenate(
                [_dot(p[-i % HP], jnp.concatenate([keys[(j - i) % HP] for j in range(HP)], axis=0).astype(BF16))
                 for i in range(HP)], axis=1)

        def mix(values):
            return _dot(jnp.concatenate(softmax(), axis=1), stack(values).astype(BF16))

        for name in order:
            if name == 'ks':
                q, k = project_rest()
                res['ks'] = k + _dot(hs[:, 2 * LANES:D], all_pairs(w_krest))
                res['q'] = q + _dot(hs[:, 2 * LANES:DF], all_pairs(w_qrest))
            elif name == 'vs':
                res[name] = _dot(hs[:, :D], all_pairs(w_vrest))
            elif name[0] in 'kv':
                pair = HP * (name[0] == 'v') + 2 * int(name[1])
                res[name] = project(pair) + project(pair + 1)
            elif name == 'r':
                res[name] = scores_rest()
            elif name == 's':
                res[name] = scores_main()
            elif name == 'px':
                res[name] = mix_rest()
            elif name == 'b2':
                res[name] = _dot(res['px'], _unpack(jnp.concatenate([w_orest[p] for p in range(HP)], axis=0)))
            elif name == 'os':
                res[name] = mix(by_head(res['vs']))
            elif name[0] == 'o':
                res[name] = mix(main_tile('v', int(name[1])))
            else:
                filler(int(name[1]))
        o = jnp.concatenate([res['o%d' % t] for t in range(NT)], axis=1) + res['b2']
        o = jnp.concatenate([o, res['os'] + pltpu.roll(res['os'], DR, 1)], axis=1)
        return o[:M], o[M:]

    def mixer_norm(h):
        return _layernorm(_layernorm(h, D), D)

    def transpose_hn(slot, c):
        hnT_s[:, c:c + LANES] = hn_s[slot, c:c + LANES, :].T[:D]

    def mixer_operands():
        ops = _strassen_lhs(hnT_s[:DH, d0], hnT_s[:DH, d1], hnT_s[DH:, d0], hnT_s[DH:, d1])
        for i, a in enumerate(ops):
            lhs_s[i] = a

    def hidden_cols(t):
        return slice(t * LANES, (t + 1) * LANES), slice(FH + t * LANES, FH + (t + 1) * LANES)

    def w1_operands(p, c1, c2):
        return _strassen_rhs(w1_s[p, d0, c1], w1_s[p, d0, c2], w1_s[p, d1, c1], w1_s[p, d1, c2])

    def accumulate(p, t, piece):
        c1, c2 = hidden_cols(t)
        rhs = w1_operands(p, c1, c2)
        n = DH // MIX_PIECES
        top, bot = slice(piece * n, (piece + 1) * n), slice(DH + piece * n, DH + (piece + 1) * n)
        c11, c12, c21, c22 = _strassen_sum(*[_dot(lhs_s[i, top], rhs[i]) for i in range(7)])
        u_s[top, c1] += c11
        u_s[top, c2] += c12
        u_s[bot, c1] += c21
        u_s[bot, c2] += c22

    def pair_cols(pair):
        return slice(2 * pair * LANES, 2 * (pair + 1) * LANES)

    def pair_body(p, mem):
        w1_copy(p).wait()

        @pl.when(p + 1 < NP)
        def _():
            x_copy(p + 1, sems.at[p]).wait()

        prev, following = jnp.maximum(p - 1, 0), jnp.minimum(p + 1, NP - 1)
        zero = jnp.minimum(p, 0)

        def mask_value_after(ref):
            return jnp.concatenate([jnp.where(p < 0, ref[zero, :SUB, :LANES], NEG)] * KG, axis=0)

        saved = {pair: [early_s[i, :, pair_cols(pair)] for i in range(len(EARLY))] for pair in range(2 * HP)}
        saved['rest'] = (early_rest_s[:seg], early_rest_s[seg:])
        now = xn_s[0], xn_s[1]
        for j in range(SPP):
            rows = slice(j * seg, (j + 1) * seg)
            x = x_s[p, rows, :]
            if j == 0:
                hn_s[p, TP - seg:, :] = mixer_norm(h_s[p, TP - seg:, :])
                for c in range(0, TP, LANES):
                    transpose_hn(p, c)
                mixer_operands()
            else:
                hn_s[p + 1, (j - 1) * seg:j * seg, :] = mixer_norm(h)
            if j == NEXT_X_AT:
                x_rows(following)
            step, tile = j % 2, j - (SPP - FH // LANES)
            ahead = None
            if step:
                ahead = x_pair(p, j + 1) if j + 1 < SPP else x_pair(following, 0)
            args = (step, mem, now, ahead, saved)
            mem, att = segment(STEP_ORDER[step], now[step], mem, main_projection(*args), rest_projection(*args),
                               functools.partial(accumulate, prev, tile) if tile >= 0 else lambda piece: None,
                               mask_value_after(hn_s))
            if step:
                now = ahead
            h = x + att
            h_s[p + 1, rows, :] = h
        xn_s[0], xn_s[1] = now
        early_rest_s[:seg], early_rest_s[seg:] = saved['rest']
        for pair in range(2 * HP):
            for i, v in enumerate(saved[pair]):
                early_s[i, :, pair_cols(pair)] = v
        return mem

    start = xn_s[0], xn_s[1]
    x7, x5 = rest_ahead(*start)
    early_rest_s[:seg], early_rest_s[seg:] = _dot(x7, all_pairs(w_rest.at[6])), _dot(x5, all_pairs(w_rest.at[4]))
    for i, r in enumerate(EARLY):
        for pair in range(2 * HP):
            early_s[i, :, pair_cols(pair)] = _dot(token_operand(r, *start), main_weights(r, pair))
    mem0 = mem0_s[...].astype(F32)
    lax.fori_loop(0, NP, pair_body, jnp.concatenate([mem0, mem0[:, DF:]], axis=1))

    def out_cols(p):
        return pl.ds(offset(2 * p, LANES), LANES), pl.ds(offset(2 * p + 1, LANES), LANES)

    def w2_operands(p, k1, k2):
        n1, n2 = out_cols(p)
        return _strassen_rhs(w2_s[k1, n1], w2_s[k1, n2], w2_s[k2, n1], w2_s[k2, n2])

    def out_store(p, c11, c12, c21, c22):
        for k, (cols, top, bot) in enumerate(zip(out_cols(p), (c11, c12), (c21, c22))):
            h = h_s[p + 1, k * LANES:(k + 1) * LANES, :].T[:D]
            y = jnp.concatenate([top, bot], axis=0)
            out_s[:, cols] = (h + (0.5 * y + b2_s[:, cols])).astype(out_s.dtype)
            out_copy(2 * p + k).start()

    def out_block(p):
        rhs = w2_operands(p, slice(0, FH), slice(FH, F))
        m = {i: _dot(g_s[i], rhs[i]) for i in OUT_ORDER}
        out_store(p, *_strassen_sum(*[m[i] for i in range(7)]))

    w2_copy.wait()
    tiles = [hidden_cols(t) for t in range(FH // LANES)]
    transpose_hn(NP, 0)
    x11, x21 = hnT_s[:DH, d0], hnT_s[DH:, d0]
    for c1, c2 in tiles:
        rhs = w1_operands(NP - 1, c1, c2)
        m3, m6 = _dot_split(x11, rhs[2], 2), _dot_split(x21 - x11, rhs[5], 2)
        u_s[:DH, c2] += m3
        u_s[DH:, c2] += m3 + m6
    hn_s[NP, TP - seg:, :] = mixer_norm(h_s[NP, TP - seg:, :])
    transpose_hn(NP, LANES)
    mixer_operands()

    acc, ready = None, []

    def drain(acc):
        k1 = slice(ready[0][1].start, ready[-1][1].stop)
        k2 = slice(ready[0][2].start, ready[-1][2].stop)
        lhs = [jnp.concatenate([r[0][i] for r in ready], axis=1) for i in range(7)]
        rhs = w2_operands(0, k1, k2)
        m = {i: _dot_split(lhs[i], rhs[i], 2) for i in (0, 1, 2, 3, 4, 6, 5)}
        prods = [m[i] for i in range(7)]
        ready.clear()
        return prods if acc is None else [a + b for a, b in zip(acc, prods)]

    for t, (c1, c2) in enumerate(tiles):
        rhs = w1_operands(NP - 1, c1, c2)
        m5, m2, m1, m4, m7 = (_dot(lhs_s[i], rhs[i]) for i in (4, 1, 0, 3, 6))
        if t and t % 2 == 0:
            acc = drain(acc)
        ops = _strassen_lhs(_gelu_twice(u_s[:DH, c1] + ((m1 + m7) + (m4 - m5))), _gelu_twice(u_s[:DH, c2] + m5),
                            _gelu_twice(u_s[DH:, c1] + (m2 + m4)), _gelu_twice(u_s[DH:, c2] + (m1 - m2)))
        for i, a in enumerate(ops):
            g_s[i, :, c1] = a
        ready.append((ops, c1, c2))
    out_store(0, *_strassen_sum(*drain(acc)))
    peeled = 1 + (NP - 1) % OUT_UNROLL
    for p in range(1, peeled):
        out_block(p)

    def out_body(i, c):
        for k in range(OUT_UNROLL):
            out_block(peeled + i * OUT_UNROLL + k)
        return c

    if NP > peeled:
        lax.fori_loop(0, (NP - peeled) // OUT_UNROLL, out_body, 0)
    for block in range(2 * NP):
        out_copy(block).wait()


@functools.partial(jax.jit, static_argnames=("A_seg_len",))
def pallas_sequential_preLN__memory_aug_recurrent_mem_tr__mixer_token_mlp__prompt_kernel(
        A_x, A_mem0, A_Wq, A_Wk, A_Wv, A_Wo, A_seg_len, B_x, B_w1, B_b1, B_w2, B_b2):
    del B_x
    B, S, D = A_x.shape
    _, H, E = A_Wq.shape
    M = A_mem0.shape[1]
    F = B_w1.shape[1]
    seg = int(A_seg_len)
    HP = H // 2
    DF = D // LANES * LANES
    DP = DF + LANES
    TP = 2 * LANES
    NP = S // TP
    assert B == 1 and M == SUB and seg == 4 * SUB and H * SUB == LANES
    assert DF == 3 * LANES and 2 * (D - DF) == LANES and S == HP * TP and F == 7 * TP
    hbm = pl.BlockSpec(memory_space=pl.ANY)
    outT = pl.pallas_call(
        functools.partial(_kernel, seg=seg, scale=E ** -0.5),
        out_shape=jax.ShapeDtypeStruct((D, S), A_x.dtype),
        in_specs=[hbm] * 10,
        out_specs=hbm,
        scratch_shapes=[
            pltpu.VMEM((HP, D, E), U32),
            pltpu.VMEM((HP, D, E), U32),
            pltpu.VMEM((HP, D, E), U32),
            pltpu.VMEM((H, D, E), BF16),
            pltpu.VMEM((NP, D, TP), BF16),
            pltpu.VMEM((NP, TP, F), BF16),
            pltpu.VMEM((F, S), BF16),
            pltpu.VMEM((M, D), BF16),
            pltpu.VMEM((F,), BF16),
            pltpu.VMEM((S,), BF16),
            pltpu.VMEM((len(PRODUCTS), 2 * H, LANES // 2, LANES), U32),
            pltpu.VMEM((7, HP, LANES // 2, LANES), U32),
            pltpu.VMEM((HP, LANES // 2, LANES), U32),
            pltpu.VMEM((HP, (D - 2 * LANES) // 2, LANES), U32),
            pltpu.VMEM((HP, D // 2, LANES), U32),
            pltpu.VMEM((HP, LANES // 2, DF), U32),
            pltpu.VMEM((len(EARLY), seg, 2 * H * LANES), F32),
            pltpu.VMEM((seg + seg // 2, HP * LANES), F32),
            pltpu.VMEM((2, seg, DP), F32),
            pltpu.VMEM((NP, TP, DP), F32),
            pltpu.VMEM((NP + 1, TP, DP), F32),
            pltpu.VMEM((NP + 1, TP, DP), F32),
            pltpu.VMEM((D, TP), F32),
            pltpu.VMEM((7, D // 2, LANES), F32),
            pltpu.VMEM((D, F), F32),
            pltpu.VMEM((7, D // 2, F // 2), F32),
            pltpu.VMEM((1, S), F32),
            pltpu.VMEM((D, S), A_x.dtype),
            pltpu.SemaphoreType.DMA((HP + 1,)),
        ],
        compiler_params=pltpu.CompilerParams(vmem_limit_bytes=110 * 2**20),
    )(
        jnp.swapaxes(A_x, 1, 2).reshape(D, S),
        A_mem0.reshape(M, D),
        A_Wq, A_Wk, A_Wv,
        jnp.swapaxes(A_Wo, 1, 2),
        B_w1, B_b1, B_w2, B_b2,
    )
    return jnp.swapaxes(outT.reshape(B, D, S), 1, 2)
```
